```python
import jax
import jax.numpy as jnp

def _softmax(x, axis=-1):
    return jax.nn.softmax(x, axis=axis)
def _gelu(x):
    return jax.nn.gelu(x, approximate=True)
def _silu(x):
    return jax.nn.silu(x)
def _sigmoid(x):
    return jax.nn.sigmoid(x)
def _layernorm(x, axis=-1, eps=1e-5):
    m = jnp.mean(x, axis=axis, keepdims=True)
    v = jnp.var(x, axis=axis, keepdims=True)
    return (x - m) / jnp.sqrt(v + eps)
def _scatter_add(tgt, idx, src, axis=0):
    return tgt.at[idx].add(src)
def _segment_sum(src, seg, n):
    return jax.ops.segment_sum(src, seg, n)
class _Rng:
    def __init__(self, key):
        self._k = key
    def _next(self):
        self._k, sub = jax.random.split(self._k)
        return sub
    def normal(self, shape):
        return jax.random.normal(self._next(), shape, dtype=jnp.bfloat16)
    def randint(self, lo, hi, shape):
        return jax.random.randint(self._next(), shape, lo, hi, dtype=jnp.int32)
    def uniform(self, shape, lo=0.0, hi=1.0):
        return jax.random.uniform(self._next(), shape, jnp.bfloat16, lo, hi)
    def permutation(self, n):
        return jax.random.permutation(self._next(), n)


kernel_name = 'sequential_preLN__compressed_kv_cla__moe_arch_mod__decode'

def setup_inputs():
    _rng = _Rng(jax.random.key(int.from_bytes(__import__("os").urandom(4), "little")))
    _w = (lambda a: (lambda t: t.astype(jnp.bfloat16) if jnp.issubdtype(t.dtype, jnp.floating) else t)(jnp.asarray(a)))
    def _A_setup():
        B, H, Sq, Sk, D, M = 1, 32, 1, 8192, 128, 512
        Dc = 4 * D
        return {
            "x": _w((lambda *s: _rng.normal(s) * 0.05)(B, Sq, M)),
            "c_kv": _w((lambda *s: _rng.normal(s) * 0.05)(B, Sk, Dc)),
            "w_q": _w((lambda *s: _rng.normal(s) * 0.05)(M, H, D) * (M ** -0.5)),
            "w_uk": _w((lambda *s: _rng.normal(s) * 0.05)(Dc, H, D) * (Dc ** -0.5)),
            "w_uv": _w((lambda *s: _rng.normal(s) * 0.05)(Dc, H, D) * (Dc ** -0.5)),
            "w_o": _w((lambda *s: _rng.normal(s) * 0.05)(H, D, M) * ((H * D) ** -0.5)),
        }
    _A_in = _A_setup()

    def _B_setup():
        B, S, D, F, C = 1, 1, 512, 1376, 1
        return {
            "x": _w((lambda *s: _rng.normal(s) * 0.05)(B, S, D)),
            "w_r": _w((lambda *s: _rng.normal(s) * 0.05)(D)),
            "w_gate": _w((lambda *s: _rng.normal(s) * 0.05)(D, F)),
            "w_up": _w((lambda *s: _rng.normal(s) * 0.05)(D, F)),
            "w_down": _w((lambda *s: _rng.normal(s) * 0.05)(F, D)),
        }
    _B_in = _B_setup()

    return {
        "A_x": _A_in["x"],
        "A_c_kv": _A_in["c_kv"],
        "A_w_q": _A_in["w_q"],
        "A_w_uk": _A_in["w_uk"],
        "A_w_uv": _A_in["w_uv"],
        "A_w_o": _A_in["w_o"],
        "B_x": _B_in["x"],
        "B_w_r": _B_in["w_r"],
        "B_w_gate": _B_in["w_gate"],
        "B_w_up": _B_in["w_up"],
        "B_w_down": _B_in["w_down"],
    }

def reference(A_x, A_c_kv, A_w_q, A_w_uk, A_w_uv, A_w_o, B_x, B_w_r, B_w_gate, B_w_up, B_w_down):
    def _A_ref(x, c_kv, w_q, w_uk, w_uv, w_o):
        B, Sq, M = x.shape[0], x.shape[1], x.shape[2]
        Sk = c_kv.shape[1]
        H, D = w_q.shape[1], w_q.shape[2]
        q = jnp.einsum("bqm,mhd->bhqd", x, w_q)
        k = jnp.einsum("bkc,chd->bhkd", c_kv, w_uk)
        v = jnp.einsum("bkc,chd->bhkd", c_kv, w_uv)
        scores = jnp.einsum("bhqd,bhkd->bhqk", q, k) * (D ** -0.5)
        off = Sk - Sq
        qi = jnp.arange(Sq)[:, None]
        kj = jnp.arange(Sk)[None, :]
        cmask = kj <= (qi + off)
        scores = jnp.where(cmask[None, None], scores, -1e9)
        p = _softmax(scores, axis=-1)
        ctx = jnp.einsum("bhqk,bhkd->bhqd", p, v)
        return jnp.einsum("bhqd,hdm->bqm", ctx, w_o)

    def _B_ref(x, w_r, w_gate, w_up, w_down):
        B, S, D = x.shape
        C = 1
        r = x @ w_r
        idx = jnp.argsort(-r, axis=-1)[:, :C]
        idx_e = jnp.repeat(idx.reshape(B, C, 1), D, axis=2)
        x_sel = jnp.take_along_axis(x, idx_e, axis=1)
        g = _silu(x_sel @ w_gate)
        u = x_sel @ w_up
        y = (g * u) @ w_down
        r_sel = _sigmoid(jnp.take_along_axis(r, idx, axis=1))
        y = y * r_sel.reshape(B, C, 1)
        b_off = (jnp.arange(B) * S).reshape(B, 1)
        flat_idx = (idx + b_off).reshape(B * C)
        zero = (x * 0.0).reshape(B * S, D)
        upd = _scatter_add(zero, flat_idx, y.reshape(B * C, D), axis=0)
        return x + upd.reshape(B, S, D)

    x = A_x
    h = x + _A_ref(_layernorm(x, axis=-1), A_c_kv, A_w_q, A_w_uk, A_w_uv, A_w_o)
    h2 = h + _B_ref(_layernorm(h, axis=-1), B_w_r, B_w_gate, B_w_up, B_w_down)
    return h2
```

```python
import functools

import jax
import jax.numpy as jnp
from jax import lax
import jax.experimental.pallas as pl
import jax.experimental.pallas.tpu as pltpu

_F32 = jnp.float32
_BF16 = jnp.bfloat16
_LANES = 128
_NT = (((1,), (1,)), ((), ()))


def _layernorm(x):
    m = jnp.mean(x, axis=-1, keepdims=True)
    d = x - m
    v = jnp.mean(d * d, axis=-1, keepdims=True)
    return d / jnp.sqrt(v + 1e-5)


def _bounds(sizes):
    out, lo = [], 0
    for s in sizes:
        out.append((lo, s))
        lo += s
    return out


def _kernel(
    x_hbm, ckv_hbm, wq_hbm, wuk_hbm, wuv_hbm, wo_hbm, wr_hbm, wg_hbm, wu_hbm, wd_hbm,
    o_ref,
    x_v, wr_v, wq_v, wuk_v, ckv_v, wuv_v, wo_v, wg_v, wu_v, wd_v,
    rows_v, ctx_v, sems,
    *, cfg,
):
    J, T, H, D = wq_v.shape
    Sk, Dc = ckv_v.shape
    M = wo_v.shape[1]
    F = wg_hbm.shape[0]
    Fp = wg_v.shape[0]
    G = cfg["G"]
    TK = cfg["TK"]
    n_kv = cfg["n_kv"]

    sem_ids = iter(range(sems.shape[0]))

    def copy(src, dst):
        return pltpu.make_async_copy(src, dst, sems.at[next(sem_ids)])

    def row_copies(src, dst, sizes):
        return [copy(src.at[pl.ds(lo, n)], dst.at[pl.ds(lo, n)]) for lo, n in _bounds(sizes)]

    cp_x = copy(x_hbm, x_v)
    cp_wq = copy(wq_hbm, wq_v)
    cp_wuk = copy(wuk_hbm, wuk_v)
    cp_kv = row_copies(ckv_hbm.at[0], ckv_v, [Sk // n_kv] * n_kv)
    cp_wuv = copy(wuv_hbm, wuv_v)
    cp_wo = row_copies(wo_hbm, wo_v, [n * D for n in cfg["wo_heads"]])
    cp_wr = copy(wr_hbm, wr_v)
    cp_wg = row_copies(wg_hbm, wg_v, cfg["wg_rows"])
    cp_wu = row_copies(wu_hbm, wu_v, cfg["wu_rows"])
    cp_wd = row_copies(wd_hbm, wd_v, cfg["wd_rows"])
    for c in [cp_x, cp_wq, cp_wuk, *cp_kv, cp_wuv, *cp_wo, cp_wr, *cp_wg, *cp_wu, *cp_wd]:
        c.start()

    if Fp > F:
        for buf in (wg_v, wu_v, wd_v):
            buf[F:Fp, :] = jnp.zeros((Fp - F, M), _BF16)

    diag = (lax.broadcasted_iota(jnp.int32, (H, J * H), 1) % H
            == lax.broadcasted_iota(jnp.int32, (H, J * H), 0))

    def tiles(w_v, t0):
        return jnp.concatenate([w_v[j, t0 + g] for g in range(G) for j in range(J)], axis=0)

    def head_contract(w_v):
        def body(i, acc):
            t0 = pl.multiple_of(i * G, G)
            r = rows_v[pl.ds(t0, G), :]
            s = jnp.concatenate(
                [jnp.where(diag, r[g:g + 1, :], 0.0) for g in range(G)], axis=1).astype(_BF16)
            return acc + jnp.dot(s, tiles(w_v, t0), preferred_element_type=_F32)
        return lax.fori_loop(0, T // G, body, jnp.zeros((H, D), _F32))

    cp_x.wait()
    x = x_v[0].astype(_F32)
    xn = _layernorm(x)
    rows_v[...] = jnp.concatenate(
        [jnp.broadcast_to(xn[:, j * T:(j + 1) * T], (H, T)) for j in range(J)], axis=0).T
    cp_wq.wait()
    q = head_contract(wq_v).astype(_BF16)

    cp_wuk.wait()

    def absorb(i, carry):
        t0 = pl.multiple_of(i * G, G)
        r = lax.dot_general(q, tiles(wuk_v, t0), _NT, preferred_element_type=_F32)
        rows_v[pl.ds(t0, G), :] = jnp.concatenate(
            [jnp.sum(jnp.where(diag, r[:, g * J * H:(g + 1) * J * H], 0.0), axis=0, keepdims=True)
             for g in range(G)], axis=0)
        return carry
    lax.fori_loop(0, T // G, absorb, 0)
    qt = rows_v[...].T
    qa = jnp.concatenate([qt[j * H:(j + 1) * H, :] for j in range(J)], axis=1)
    qa = (qa * (D ** -0.5)).astype(_BF16)

    def attend(i, carry):
        m, l, acc = carry
        kv = ckv_v[pl.ds(pl.multiple_of(i * TK, TK), TK), :]
        s = lax.dot_general(qa, kv, _NT, preferred_element_type=_F32)
        m_new = jnp.maximum(m, jnp.max(s, axis=-1, keepdims=True))
        alpha = jnp.exp(m - m_new)
        p = jnp.exp(s - m_new)
        l = alpha * l + jnp.sum(p, axis=-1, keepdims=True)
        acc = alpha * acc + jnp.dot(p.astype(_BF16), kv, preferred_element_type=_F32)
        return m_new, l, acc

    carry = (jnp.full((H, 1), -jnp.inf, _F32), jnp.zeros((H, 1), _F32), jnp.zeros((H, Dc), _F32))
    steps = Sk // n_kv // TK
    for c in range(n_kv):
        cp_kv[c].wait()
        carry = lax.fori_loop(c * steps, (c + 1) * steps, attend, carry)
    _, l, acc = carry
    lat = acc / l

    rows_v[...] = jnp.concatenate([lat[:, j * T:(j + 1) * T] for j in range(J)], axis=0).T
    cp_wuv.wait()
    ctx_v[...] = head_contract(wuv_v)

    R = 16
    attn = jnp.zeros((R, M), _F32)
    for c, (h0, nh) in zip(cp_wo, _bounds(cfg["wo_heads"])):
        a = jnp.concatenate(
            [jnp.broadcast_to(ctx_v[h:h + 1, :], (R, D)) for h in range(h0, h0 + nh)], axis=1)
        c.wait()
        attn += jnp.dot(a.astype(_BF16), wo_v[h0 * D:(h0 + nh) * D, :], preferred_element_type=_F32)

    h = x + attn
    hn = _layernorm(h)
    hb = hn.astype(_BF16)

    cp_wr.wait()
    r = jnp.sum(hn * wr_v[...].astype(_F32).reshape(1, M), axis=-1, keepdims=True)
    gate = jax.nn.sigmoid(r)

    def padded(sizes):
        b = _bounds(sizes)
        return b[:-1] + [(b[-1][0], Fp - b[-1][0])]

    def project(cps, buf, sizes):
        out = []
        for c, (lo, n) in zip(cps, padded(sizes)):
            c.wait()
            out.append(lax.dot_general(hb, buf[lo:lo + n, :], _NT, preferred_element_type=_F32))
        return jnp.concatenate(out, axis=1)

    g = jax.nn.silu(project(cp_wg, wg_v, cfg["wg_rows"]))
    act = (g * project(cp_wu, wu_v, cfg["wu_rows"])).astype(_BF16)

    y = jnp.zeros((R, M), _F32)
    for c, (lo, n) in zip(cp_wd, padded(cfg["wd_rows"])):
        c.wait()
        y += jnp.dot(act[:, lo:lo + n], wd_v[lo:lo + n, :], preferred_element_type=_F32)

    upd = hn * 0.0 + y * gate
    o_ref[0] = (h + (hn + upd))[0:1, :].astype(o_ref.dtype)


_CFG = dict(
    G=8,
    TK=1024,
    n_kv=4,
    wo_heads=(16, 12, 4),
    wg_rows=(1376,),
    wu_rows=(768, 608),
    wd_rows=(768, 384, 224),
)


def _call(A_x, A_c_kv, A_w_q, A_w_uk, A_w_uv, A_w_o, B_w_r, B_w_gate, B_w_up, B_w_down, cfg):
    B, Sq, M = A_x.shape
    _, Sk, Dc = A_c_kv.shape
    _, H, D = A_w_q.shape
    F = B_w_down.shape[0]
    assert B == 1 and Sq == 1 and M == Dc and D == _LANES and _LANES % H == 0
    J = _LANES // H
    T = Dc // J
    assert T == _LANES
    Fp = pl.cdiv(F, _LANES) * _LANES
    n_sems = (5 + cfg["n_kv"] + len(cfg["wo_heads"]) + len(cfg["wg_rows"])
              + len(cfg["wu_rows"]) + len(cfg["wd_rows"]))
    hbm = pl.BlockSpec(memory_space=pltpu.MemorySpace.HBM)
    slabs = (J, T, H, D)
    return pl.pallas_call(
        functools.partial(_kernel, cfg=cfg),
        in_specs=[hbm] * 10,
        out_specs=pl.BlockSpec(memory_space=pltpu.MemorySpace.VMEM),
        out_shape=jax.ShapeDtypeStruct((B, Sq, M), A_x.dtype),
        scratch_shapes=[
            pltpu.VMEM((B, Sq, M), _BF16),
            pltpu.VMEM((M,), _BF16),
            pltpu.VMEM(slabs, _BF16),
            pltpu.VMEM(slabs, _BF16),
            pltpu.VMEM((Sk, Dc), _BF16),
            pltpu.VMEM(slabs, _BF16),
            pltpu.VMEM((H * D, M), _BF16),
            pltpu.VMEM((Fp, M), _BF16),
            pltpu.VMEM((Fp, M), _BF16),
            pltpu.VMEM((Fp, M), _BF16),
            pltpu.VMEM((T, J * H), _F32),
            pltpu.VMEM((H, D), _F32),
            pltpu.SemaphoreType.DMA((n_sems,)),
        ],
        compiler_params=pltpu.CompilerParams(
            vmem_limit_bytes=64 * 1024 * 1024,
            disable_semaphore_checks=cfg.get("no_sem_checks", True),
        ),
    )(
        A_x, A_c_kv,
        A_w_q.reshape(slabs), A_w_uk.reshape(slabs), A_w_uv.reshape(slabs),
        A_w_o.reshape(H * D, M),
        B_w_r,
        B_w_gate.T, B_w_up.T, B_w_down,
    )


@jax.jit
def pallas_sequential_preLN__compressed_kv_cla__moe_arch_mod__decode_kernel(
    A_x: jax.Array,
    A_c_kv: jax.Array,
    A_w_q: jax.Array,
    A_w_uk: jax.Array,
    A_w_uv: jax.Array,
    A_w_o: jax.Array,
    B_x: jax.Array,
    B_w_r: jax.Array,
    B_w_gate: jax.Array,
    B_w_up: jax.Array,
    B_w_down: jax.Array,
):
    del B_x
    return _call(A_x, A_c_kv, A_w_q, A_w_uk, A_w_uv, A_w_o,
                 B_w_r, B_w_gate, B_w_up, B_w_down, _CFG)
```

```python
import functools

import jax
import jax.numpy as jnp
from jax import lax
import jax.experimental.pallas as pl
import jax.experimental.pallas.tpu as pltpu

_F32 = jnp.float32
_BF16 = jnp.bfloat16
_LANES = 128
_NT = (((1,), (1,)), ((), ()))

_REGIONS = 8
_PER_UNIT = 4
_PIECE = 32
_AHEAD = 3
_RING = 4
_ROWS = 16


def _layernorm(x):
    m = jnp.mean(x, axis=-1, keepdims=True)
    d = x - m
    v = jnp.mean(d * d, axis=-1, keepdims=True)
    return d / jnp.sqrt(v + 1e-5)


def _bounds(sizes):
    out, lo = [], 0
    for s in sizes:
        out.append((lo, s))
        lo += s
    return out


def _kernel(
    x_hbm, ckv_hbm, wq_hbm, wuk_hbm, wuv_hbm, wo_hbm, wr_hbm, wg_hbm, wu_hbm, wd_hbm,
    o_ref,
    x_v, wr_v, wq_v, wuk_v, ckv_v, wuv_v, wo_v, wg_v, wu_v, wd_v,
    rows_v, ctx_v, ring_sems, io_sems, ffn_sems,
    *, cfg,
):
    NU, _, TU, H, D = wq_v.shape
    NKV, TK, Dc = ckv_v.shape
    M = wo_v.shape[2]
    F = wg_hbm.shape[0]
    Fp = wg_v.shape[0]
    J = _LANES // H
    T = Dc // J
    G = cfg["G"]
    order = cfg["order"]

    def slab_piece(w_hbm, w_v):
        n = TU // _PER_UNIT
        return lambda u, r, i: (w_hbm.at[pl.ds(r * (NU * TU) + u * TU + i * n, n)],
                                w_v.at[u, r, pl.ds(i * n, n)])

    def kv_piece(u, r, i):
        blk, s = u // NU, u % NU
        row = (blk * _REGIONS + r) * (NU * _PER_UNIT * _PIECE) + (s * _PER_UNIT + i) * _PIECE
        return (ckv_hbm.at[0, pl.ds(pl.multiple_of(row, _PIECE), _PIECE)],
                ckv_v.at[u, pl.ds((r * _PER_UNIT + i) * _PIECE, _PIECE)])

    def wo_piece(u, r, i):
        return (wo_hbm.at[r * NU + u, pl.ds(i * _PIECE, _PIECE)],
                wo_v.at[u, pl.ds((r * _PER_UNIT + i) * _PIECE, _PIECE)])

    phases = [(slab_piece(wq_hbm, wq_v), wq_v), (slab_piece(wuk_hbm, wuk_v), wuk_v),
              (kv_piece, ckv_v), (slab_piece(wuv_hbm, wuv_v), wuv_v), (wo_piece, wo_v)]
    assert all(buf.shape[0] % _RING == 0 for _, buf in phases)

    def start_unit(p, u):
        for i in range(_PER_UNIT):
            for k, r in enumerate(order):
                src, dst = phases[p][0](u, r, i)
                pltpu.make_async_copy(src, dst, ring_sems.at[u % _RING]).start(priority=k % 2)

    n_pieces = F // _PIECE
    per = pl.cdiv(n_pieces, cfg["ffn_regions"])
    hidden = [r * per + i for i in range(per) for r in range(cfg["ffn_regions"])
              if r * per + i < n_pieces]
    gu_units, wd_units = _bounds(cfg["gu_pieces"]), _bounds(cfg["wd_pieces"])
    ffn_queue, ffn_ends = [], []
    for k, (lo, n) in enumerate(gu_units):
        for i in range(lo, lo + n):
            ffn_queue += [(wg_hbm, wg_v, i, 2 * k), (wu_hbm, wu_v, i, 2 * k + 1)]
        ffn_ends.append(len(ffn_queue))
    for k, (lo, n) in enumerate(wd_units):
        ffn_queue += [(wd_hbm, wd_v, i, 2 * len(gu_units) + k) for i in range(lo, lo + n)]
        ffn_ends.append(len(ffn_queue))
    unit_pieces = _REGIONS * _PER_UNIT

    def start_ffn(lo, hi):
        for k in range(lo, min(hi, len(ffn_queue))):
            src, dst, i, s = ffn_queue[k]
            pltpu.make_async_copy(src.at[pl.ds(hidden[i] * _PIECE, _PIECE)],
                                  dst.at[pl.ds(i * _PIECE, _PIECE)],
                                  ffn_sems.at[s]).start(priority=k % 2)

    def wait_rows(buf, lo, n, sem):
        rows = buf.at[pl.ds(lo * _PIECE, n * _PIECE)]
        pltpu.make_async_copy(rows, rows, sem).wait()

    def advance(p, u):
        buf = phases[p][1]
        n = buf.shape[0]
        pl.when(u + _AHEAD < n)(lambda: start_unit(p, u + _AHEAD))
        if p + 1 < len(phases):
            pl.when(u + _AHEAD >= n)(lambda: start_unit(p + 1, u + _AHEAD - n))
        else:
            for k in range(_AHEAD):
                pl.when(u + _AHEAD == n + k)(
                    functools.partial(start_ffn, k * unit_pieces, (k + 1) * unit_pieces))
        pltpu.make_async_copy(buf.at[u], buf.at[u], ring_sems.at[u % _RING]).wait()

    cp_x = pltpu.make_async_copy(x_hbm, x_v, io_sems.at[0])
    cp_wr = pltpu.make_async_copy(wr_hbm, wr_v, io_sems.at[1])
    cp_x.start(priority=0)
    cp_wr.start(priority=1)
    lax.fori_loop(0, _AHEAD, lambda u, c: start_unit(0, u), None)

    if Fp > F:
        for buf in (wg_v, wu_v, wd_v):
            buf[F:Fp, :] = jnp.zeros((Fp - F, M), _BF16)

    diag = (lax.broadcasted_iota(jnp.int32, (H, J * H), 1) % H
            == lax.broadcasted_iota(jnp.int32, (H, J * H), 0))
    halves = _REGIONS // J
    per_half = TU // G

    def tile_group(w_v, u, k):
        half, t0 = k // per_half, (k % per_half) * G
        w = jnp.concatenate(
            [w_v[u, halves * j + half, t0 + g] for g in range(G) for j in range(J)], axis=0)
        return w, pl.multiple_of(half * (NU * TU) + u * TU + t0, G)

    def head_contract(p):
        def unit(u, acc):
            advance(p, u)

            def group(k, acc):
                w, t = tile_group(phases[p][1], u, k)
                r = rows_v[pl.ds(t, G), :]
                s = jnp.concatenate(
                    [jnp.where(diag, r[g:g + 1, :], 0.0) for g in range(G)], axis=1)
                return acc + jnp.dot(s.astype(_BF16), w, preferred_element_type=_F32)
            return lax.fori_loop(0, halves * per_half, group, acc)
        return lax.fori_loop(0, NU, unit, jnp.zeros((H, D), _F32))

    cp_x.wait()
    x = x_v[0].astype(_F32)
    xn = _layernorm(x)
    rows_v[...] = jnp.concatenate(
        [jnp.broadcast_to(xn[:, j * T:(j + 1) * T], (H, T)) for j in range(J)], axis=0).T
    q = head_contract(0).astype(_BF16)

    def absorb(u, carry):
        advance(1, u)

        def group(k, carry):
            w, t = tile_group(wuk_v, u, k)
            r = lax.dot_general(q, w, _NT, preferred_element_type=_F32)
            rows_v[pl.ds(t, G), :] = jnp.concatenate(
                [jnp.sum(jnp.where(diag, r[:, g * J * H:(g + 1) * J * H], 0.0),
                         axis=0, keepdims=True) for g in range(G)], axis=0)
            return carry
        return lax.fori_loop(0, halves * per_half, group, carry)
    lax.fori_loop(0, NU, absorb, None)
    qt = rows_v[...].T
    qa = jnp.concatenate([qt[j * H:(j + 1) * H, :] for j in range(J)], axis=1)
    qa = (qa * (D ** -0.5)).astype(_BF16)

    def attend(u, carry):
        m, l, acc = carry
        advance(2, u)
        s = lax.dot_general(qa, ckv_v[u], _NT, preferred_element_type=_F32)
        m_new = jnp.maximum(m, jnp.max(s, axis=-1, keepdims=True))
        alpha = jnp.exp(m - m_new)
        p = jnp.exp(s - m_new)
        l = alpha * l + jnp.sum(p, axis=-1, keepdims=True)
        acc = alpha * acc + jnp.dot(p.astype(_BF16), ckv_v[u], preferred_element_type=_F32)
        return m_new, l, acc

    _, l, acc = lax.fori_loop(
        0, NKV, attend,
        (jnp.full((H, 1), -jnp.inf, _F32), jnp.zeros((H, 1), _F32), jnp.zeros((H, Dc), _F32)))
    lat = acc / l

    rows_v[...] = jnp.concatenate([lat[:, j * T:(j + 1) * T] for j in range(J)], axis=0).T
    ctx_v[...] = head_contract(3)

    def out_proj(u, attn):
        advance(4, u)
        for r in range(_REGIONS):
            a = jnp.broadcast_to(ctx_v[pl.ds(r * NU + u, 1), :], (_ROWS, D)).astype(_BF16)
            attn += jnp.dot(a, wo_v[u, r * D:(r + 1) * D, :], preferred_element_type=_F32)
        return attn
    attn = lax.fori_loop(0, NU, out_proj, jnp.zeros((_ROWS, M), _F32))

    h = x + attn
    hn = _layernorm(h)
    hb = hn.astype(_BF16)

    cp_wr.wait()
    r = jnp.sum(hn * wr_v[...].astype(_F32).reshape(1, M), axis=-1, keepdims=True)
    gate = jax.nn.sigmoid(r)

    queued = _AHEAD * unit_pieces

    def top_up(k):
        nonlocal queued
        target = ffn_ends[k] + _AHEAD * unit_pieces
        start_ffn(queued, target)
        queued = max(queued, target)

    def tile_rows(lo, n):
        hi = (lo + n) * _PIECE
        return slice(lo * _PIECE, Fp if hi == F else hi)

    act = []
    for k, (lo, n) in enumerate(gu_units):
        top_up(k)
        wait_rows(wg_v, lo, n, ffn_sems.at[2 * k])
        wait_rows(wu_v, lo, n, ffn_sems.at[2 * k + 1])
        g = lax.dot_general(hb, wg_v[tile_rows(lo, n), :], _NT, preferred_element_type=_F32)
        up = lax.dot_general(hb, wu_v[tile_rows(lo, n), :], _NT, preferred_element_type=_F32)
        act.append((jax.nn.silu(g) * up).astype(_BF16))
    act = jnp.concatenate(act, axis=1)

    y = jnp.zeros((_ROWS, M), _F32)
    for k, (lo, n) in enumerate(wd_units):
        top_up(len(gu_units) + k)
        wait_rows(wd_v, lo, n, ffn_sems.at[2 * len(gu_units) + k])
        rows = tile_rows(lo, n)
        for c in range(rows.start, rows.stop, 2 * _LANES):
            e = min(c + 2 * _LANES, rows.stop)
            y += jnp.dot(act[:, c:e], wd_v[c:e, :], preferred_element_type=_F32)

    upd = hn * 0.0 + y * gate
    o_ref[0] = (h + (hn + upd))[0:1, :].astype(o_ref.dtype)


_CFG = dict(
    G=16,
    order=(0, 4, 2, 6, 1, 5, 3, 7),
    ffn_regions=4,
    gu_pieces=(16, 16, 11),
    wd_pieces=(20, 12, 8, 3),
)


def _call(A_x, A_c_kv, A_w_q, A_w_uk, A_w_uv, A_w_o, B_w_r, B_w_gate, B_w_up, B_w_down, cfg):
    B, Sq, M = A_x.shape
    _, Sk, Dc = A_c_kv.shape
    _, H, D = A_w_q.shape
    F = B_w_down.shape[0]
    unit_rows = _REGIONS * _PER_UNIT * _PIECE
    NU = H * D // unit_rows
    assert B == 1 and Sq == 1 and M == Dc and D == _LANES and Dc * H == _LANES * _LANES
    assert D == _PER_UNIT * _PIECE and Sk % (NU * unit_rows) == 0 and F % _PIECE == 0
    Fp = pl.cdiv(F, _LANES) * _LANES
    slabs = (NU, _REGIONS, Dc // (NU * _REGIONS), H, D)
    hbm = pl.BlockSpec(memory_space=pltpu.MemorySpace.HBM)
    return pl.pallas_call(
        functools.partial(_kernel, cfg=cfg),
        in_specs=[hbm] * 10,
        out_specs=pl.BlockSpec(memory_space=pltpu.MemorySpace.VMEM),
        out_shape=jax.ShapeDtypeStruct((B, Sq, M), A_x.dtype),
        scratch_shapes=[
            pltpu.VMEM((B, Sq, M), _BF16),
            pltpu.VMEM((M,), _BF16),
            pltpu.VMEM(slabs, _BF16),
            pltpu.VMEM(slabs, _BF16),
            pltpu.VMEM((Sk // unit_rows, unit_rows, Dc), _BF16),
            pltpu.VMEM(slabs, _BF16),
            pltpu.VMEM((NU, unit_rows, M), _BF16),
            pltpu.VMEM((Fp, M), _BF16),
            pltpu.VMEM((Fp, M), _BF16),
            pltpu.VMEM((Fp, M), _BF16),
            pltpu.VMEM((_LANES, _LANES), _F32),
            pltpu.VMEM((H, D), _F32),
            pltpu.SemaphoreType.DMA((_RING,)),
            pltpu.SemaphoreType.DMA((2,)),
            pltpu.SemaphoreType.DMA((2 * len(cfg["gu_pieces"]) + len(cfg["wd_pieces"]),)),
        ],
        compiler_params=pltpu.CompilerParams(
            vmem_limit_bytes=64 * 1024 * 1024,
            disable_semaphore_checks=cfg.get("no_sem_checks", True),
            disable_bounds_checks=cfg.get("no_bounds_checks", True),
        ),
    )(
        A_x, A_c_kv, A_w_q, A_w_uk, A_w_uv, A_w_o, B_w_r,
        B_w_gate.T, B_w_up.T, B_w_down,
    )


@jax.jit
def pallas_sequential_preLN__compressed_kv_cla__moe_arch_mod__decode_kernel(
    A_x: jax.Array,
    A_c_kv: jax.Array,
    A_w_q: jax.Array,
    A_w_uk: jax.Array,
    A_w_uv: jax.Array,
    A_w_o: jax.Array,
    B_x: jax.Array,
    B_w_r: jax.Array,
    B_w_gate: jax.Array,
    B_w_up: jax.Array,
    B_w_down: jax.Array,
):
    del B_x
    return _call(A_x, A_c_kv, A_w_q, A_w_uk, A_w_uv, A_w_o,
                 B_w_r, B_w_gate, B_w_up, B_w_down, _CFG)
```

```python
import functools

import jax
import jax.numpy as jnp
from jax import lax
import jax.experimental.pallas as pl
import jax.experimental.pallas.tpu as pltpu

_F32 = jnp.float32
_BF16 = jnp.bfloat16
_LANES = 128
_NT = (((1,), (1,)), ((), ()))

_REGIONS = 8
_PER_UNIT = 4
_PIECE = 32
_AHEAD = 3
_RING = 4
_ROWS = 16


def _layernorm(x):
    m = jnp.mean(x, axis=-1, keepdims=True)
    d = x - m
    v = jnp.mean(d * d, axis=-1, keepdims=True)
    return d / jnp.sqrt(v + 1e-5)


def _bounds(sizes):
    out, lo = [], 0
    for s in sizes:
        out.append((lo, s))
        lo += s
    return out


def _kernel(
    x_hbm, ckv_hbm, wq_hbm, wuk_hbm, wuv_hbm, wo_hbm, wr_hbm, wg_hbm, wu_hbm, wd_hbm,
    o_ref,
    x_v, wr_v, wq_v, wuk_v, ckv_v, wuv_v, wo_v, wg_v, wu_v, wd_v,
    rows_v, ctx_v, ring_sems, io_sems, ffn_sems,
    *, cfg,
):
    NU, _, TU, H, D = wq_v.shape
    NKV, TK, Dc = ckv_v.shape
    M = wo_v.shape[2]
    F = wg_hbm.shape[0]
    Fp = wg_v.shape[0]
    J = _LANES // H
    T = Dc // J
    G = cfg["G"]
    order = cfg["order"]

    def slab_piece(w_hbm, w_v):
        n = TU // _PER_UNIT
        return lambda u, r, i: (w_hbm.at[pl.ds(r * (NU * TU) + u * TU + i * n, n)],
                                w_v.at[u, r, pl.ds(i * n, n)])

    def kv_piece(u, r, i):
        row = (r * NKV + u) * (_PER_UNIT * _PIECE) + i * _PIECE
        return (ckv_hbm.at[0, pl.ds(pl.multiple_of(row, _PIECE), _PIECE)],
                ckv_v.at[u, pl.ds((r * _PER_UNIT + i) * _PIECE, _PIECE)])

    def wo_piece(u, r, i):
        return (wo_hbm.at[r * NU + u, pl.ds(i * _PIECE, _PIECE)],
                wo_v.at[u, pl.ds((r * _PER_UNIT + i) * _PIECE, _PIECE)])

    phases = [(slab_piece(wq_hbm, wq_v), wq_v), (slab_piece(wuk_hbm, wuk_v), wuk_v),
              (kv_piece, ckv_v), (slab_piece(wuv_hbm, wuv_v), wuv_v), (wo_piece, wo_v)]
    assert all(buf.shape[0] % _RING == 0 for _, buf in phases)

    def start_unit(p, u):
        for i in range(_PER_UNIT):
            for k, r in enumerate(order):
                src, dst = phases[p][0](u, r, i)
                pltpu.make_async_copy(src, dst, ring_sems.at[u % _RING]).start(priority=k % 2)

    n_pieces = F // _PIECE
    per = cfg["ffn_stride"]
    hidden = [j for i in range(per) for j in range(i, n_pieces, per)]
    gu_units = _bounds(cfg["gu_pieces"])
    wd_units = _bounds(cfg["wd_pieces"] + cfg["wd_tail_pieces"])
    ffn_queue, ffn_ends = [], []
    for k, (lo, n) in enumerate(gu_units):
        for i in range(lo, lo + n):
            ffn_queue += [(wg_hbm, wg_v, i, 2 * k), (wu_hbm, wu_v, i, 2 * k + 1)]
        ffn_ends.append(len(ffn_queue))
    for k, (lo, n) in enumerate(wd_units):
        ffn_queue += [(wd_hbm, wd_v, i, 2 * len(gu_units) + k) for i in range(lo, lo + n)]
        ffn_ends.append(len(ffn_queue))
    unit_pieces = _REGIONS * _PER_UNIT

    def start_ffn(lo, hi):
        for k in range(lo, min(hi, len(ffn_queue))):
            src, dst, i, s = ffn_queue[k]
            pltpu.make_async_copy(src.at[pl.ds(hidden[i] * _PIECE, _PIECE)],
                                  dst.at[pl.ds(i * _PIECE, _PIECE)],
                                  ffn_sems.at[s]).start(priority=k % 2)

    def wait_rows(buf, lo, n, sem):
        rows = buf.at[pl.ds(lo * _PIECE, n * _PIECE)]
        pltpu.make_async_copy(rows, rows, sem).wait()

    def advance(p, u):
        buf = phases[p][1]
        n = buf.shape[0]
        pl.when(u + _AHEAD < n)(lambda: start_unit(p, u + _AHEAD))
        if p + 1 < len(phases):
            pl.when(u + _AHEAD >= n)(lambda: start_unit(p + 1, u + _AHEAD - n))
        else:
            for k in range(_AHEAD):
                pl.when(u + _AHEAD == n + k)(
                    functools.partial(start_ffn, k * unit_pieces, (k + 1) * unit_pieces))
        pltpu.make_async_copy(buf.at[u], buf.at[u], ring_sems.at[u % _RING]).wait()

    cp_x = pltpu.make_async_copy(x_hbm, x_v, io_sems.at[0])
    cp_wr = pltpu.make_async_copy(wr_hbm, wr_v, io_sems.at[1])
    cp_x.start(priority=0)
    cp_wr.start(priority=1)
    lax.fori_loop(0, _AHEAD, lambda u, c: start_unit(0, u), None)

    if Fp > F:
        for buf in (wg_v, wu_v, wd_v):
            buf[F:Fp, :] = jnp.zeros((Fp - F, M), _BF16)

    diag = (lax.broadcasted_iota(jnp.int32, (H, J * H), 1) % H
            == lax.broadcasted_iota(jnp.int32, (H, J * H), 0))
    halves = _REGIONS // J
    per_half = TU // G

    def tile_group(w_v, u, k):
        half, t0 = k // per_half, (k % per_half) * G
        w = jnp.concatenate(
            [w_v[u, halves * j + half, t0 + g] for g in range(G) for j in range(J)], axis=0)
        return w, pl.multiple_of(half * (NU * TU) + u * TU + t0, G)

    def head_contract(p):
        def unit(u, acc):
            advance(p, u)

            def group(k, acc):
                w, t = tile_group(phases[p][1], u, k)
                r = rows_v[pl.ds(t, G), :]
                s = jnp.concatenate(
                    [jnp.where(diag, r[g:g + 1, :], 0.0) for g in range(G)], axis=1)
                return acc + jnp.dot(s.astype(_BF16), w, preferred_element_type=_F32)
            return lax.fori_loop(0, halves * per_half, group, acc)
        return lax.fori_loop(0, NU, unit, jnp.zeros((H, D), _F32))

    cp_x.wait()
    x = x_v[0].astype(_F32)
    xn = _layernorm(x)
    rows_v[...] = jnp.concatenate(
        [jnp.broadcast_to(xn[:, j * T:(j + 1) * T], (H, T)) for j in range(J)], axis=0).T
    q = head_contract(0).astype(_BF16)

    def absorb(u, carry):
        advance(1, u)

        def group(k, carry):
            w, t = tile_group(wuk_v, u, k)
            r = lax.dot_general(q, w, _NT, preferred_element_type=_F32)
            rows_v[pl.ds(t, G), :] = jnp.concatenate(
                [jnp.sum(jnp.where(diag, r[:, g * J * H:(g + 1) * J * H], 0.0),
                         axis=0, keepdims=True) for g in range(G)], axis=0)
            return carry
        return lax.fori_loop(0, halves * per_half, group, carry)
    lax.fori_loop(0, NU, absorb, None)
    qt = rows_v[...].T
    qa = jnp.concatenate([qt[j * H:(j + 1) * H, :] for j in range(J)], axis=1)
    qa = (qa * (D ** -0.5)).astype(_BF16)

    def attend(u, carry):
        m, l, acc = carry
        advance(2, u)
        s = lax.dot_general(qa, ckv_v[u], _NT, preferred_element_type=_F32)
        m_new = jnp.maximum(m, jnp.max(s, axis=-1, keepdims=True))
        alpha = jnp.exp(m - m_new)
        p = jnp.exp(s - m_new)
        l = alpha * l + jnp.sum(p, axis=-1, keepdims=True)
        acc = alpha * acc + jnp.dot(p.astype(_BF16), ckv_v[u], preferred_element_type=_F32)
        return m_new, l, acc

    _, l, acc = lax.fori_loop(
        0, NKV, attend,
        (jnp.full((H, 1), -jnp.inf, _F32), jnp.zeros((H, 1), _F32), jnp.zeros((H, Dc), _F32)))
    lat = acc / l

    rows_v[...] = jnp.concatenate([lat[:, j * T:(j + 1) * T] for j in range(J)], axis=0).T
    ctx_v[...] = head_contract(3)

    def out_proj(u, attn):
        advance(4, u)
        for r in range(_REGIONS):
            a = jnp.broadcast_to(ctx_v[pl.ds(r * NU + u, 1), :], (_ROWS, D)).astype(_BF16)
            attn += jnp.dot(a, wo_v[u, r * D:(r + 1) * D, :], preferred_element_type=_F32)
        return attn
    attn = lax.fori_loop(0, NU, out_proj, jnp.zeros((_ROWS, M), _F32))

    h = x + attn
    hn = _layernorm(h)
    hb = hn.astype(_BF16)

    cp_wr.wait()
    r = jnp.sum(hn * wr_v[...].astype(_F32).reshape(1, M), axis=-1, keepdims=True)
    gate = jax.nn.sigmoid(r)

    queued = _AHEAD * unit_pieces

    def top_up(k):
        nonlocal queued
        target = ffn_ends[k] + _AHEAD * unit_pieces
        start_ffn(queued, target)
        queued = max(queued, target)

    def tile_rows(lo, n):
        hi = (lo + n) * _PIECE
        return slice(lo * _PIECE, Fp if hi == F else hi)

    act = []
    for k, (lo, n) in enumerate(gu_units):
        top_up(k)
        wait_rows(wg_v, lo, n, ffn_sems.at[2 * k])
        wait_rows(wu_v, lo, n, ffn_sems.at[2 * k + 1])
        g = lax.dot_general(hb, wg_v[tile_rows(lo, n), :], _NT, preferred_element_type=_F32)
        up = lax.dot_general(hb, wu_v[tile_rows(lo, n), :], _NT, preferred_element_type=_F32)
        act.append((jax.nn.silu(g) * up).astype(_BF16))
    act = jnp.concatenate(act, axis=1)

    def wait_down(k):
        top_up(len(gu_units) + k)
        wait_rows(wd_v, *wd_units[k], ffn_sems.at[2 * len(gu_units) + k])

    n_mxu = len(cfg["wd_pieces"])
    split = sum(cfg["wd_pieces"]) * _PIECE
    coef = act[0:1, split:].astype(_F32) * gate[0:1]
    col = jnp.concatenate(
        [jnp.broadcast_to(coef[:, c:c + _LANES], (_LANES, _LANES)).T
         for c in range(0, Fp - split, _LANES)], axis=0)

    y = jnp.zeros((_ROWS, M), _F32)
    for k, (lo, n) in enumerate(wd_units[:n_mxu]):
        wait_down(k)
        for c in range(lo * _PIECE, (lo + n) * _PIECE, 2 * _LANES):
            e = min(c + 2 * _LANES, (lo + n) * _PIECE)
            y += jnp.dot(act[:, c:e], wd_v[c:e, :], preferred_element_type=_F32)

    upd = hn * 0.0 + y * gate
    first = lax.broadcasted_iota(jnp.int32, (8, M), 0) == 0
    out = jnp.where(first, (h + (hn + upd))[0:8], 0.0)
    out = [out[:, c:c + _LANES] for c in range(0, M, _LANES)]
    for k, (lo, n) in list(enumerate(wd_units))[n_mxu:]:
        wait_down(k)
        for c in range(lo * _PIECE, (lo + n) * _PIECE, 16):
            w = wd_v[c:c + 16, :].astype(_F32)
            a = col[c - split:c - split + 16]
            for j in range(M // _LANES):
                t = w[:, j * _LANES:(j + 1) * _LANES] * a
                out[j] = out[j] + (t[0:8] + t[8:16])
    o_ref[0] = jnp.sum(jnp.concatenate(out, axis=1), axis=0, keepdims=True).astype(o_ref.dtype)


_CFG = dict(
    G=16,
    order=(0, 4, 2, 6, 1, 5, 3, 7),
    ffn_stride=16,
    gu_pieces=(16, 16, 11),
    wd_pieces=(24,),
    wd_tail_pieces=(8, 6, 5),
)


def _call(A_x, A_c_kv, A_w_q, A_w_uk, A_w_uv, A_w_o, B_w_r, B_w_gate, B_w_up, B_w_down, cfg):
    B, Sq, M = A_x.shape
    _, Sk, Dc = A_c_kv.shape
    _, H, D = A_w_q.shape
    F = B_w_down.shape[0]
    unit_rows = _REGIONS * _PER_UNIT * _PIECE
    NU = H * D // unit_rows
    assert B == 1 and Sq == 1 and M == Dc and D == _LANES and Dc * H == _LANES * _LANES
    assert D == _PER_UNIT * _PIECE and Sk % (NU * unit_rows) == 0 and F % _PIECE == 0
    Fp = pl.cdiv(F, _LANES) * _LANES
    slabs = (NU, _REGIONS, Dc // (NU * _REGIONS), H, D)
    hbm = pl.BlockSpec(memory_space=pltpu.MemorySpace.HBM)
    return pl.pallas_call(
        functools.partial(_kernel, cfg=cfg),
        in_specs=[hbm] * 10,
        out_specs=pl.BlockSpec(memory_space=pltpu.MemorySpace.VMEM),
        out_shape=jax.ShapeDtypeStruct((B, Sq, M), A_x.dtype),
        scratch_shapes=[
            pltpu.VMEM((B, Sq, M), _BF16),
            pltpu.VMEM((M,), _BF16),
            pltpu.VMEM(slabs, _BF16),
            pltpu.VMEM(slabs, _BF16),
            pltpu.VMEM((Sk // unit_rows, unit_rows, Dc), _BF16),
            pltpu.VMEM(slabs, _BF16),
            pltpu.VMEM((NU, unit_rows, M), _BF16),
            pltpu.VMEM((Fp, M), _BF16),
            pltpu.VMEM((Fp, M), _BF16),
            pltpu.VMEM((Fp, M), _BF16),
            pltpu.VMEM((_LANES, _LANES), _F32),
            pltpu.VMEM((H, D), _F32),
            pltpu.SemaphoreType.DMA((_RING,)),
            pltpu.SemaphoreType.DMA((2,)),
            pltpu.SemaphoreType.DMA(
                (2 * len(cfg["gu_pieces"]) + len(cfg["wd_pieces"] + cfg["wd_tail_pieces"]),)),
        ],
        compiler_params=pltpu.CompilerParams(
            vmem_limit_bytes=64 * 1024 * 1024,
            disable_semaphore_checks=cfg.get("no_sem_checks", True),
            disable_bounds_checks=cfg.get("no_bounds_checks", True),
        ),
    )(
        A_x, A_c_kv, A_w_q, A_w_uk, A_w_uv, A_w_o, B_w_r,
        B_w_gate.T, B_w_up.T, B_w_down,
    )


@jax.jit
def pallas_sequential_preLN__compressed_kv_cla__moe_arch_mod__decode_kernel(
    A_x: jax.Array,
    A_c_kv: jax.Array,
    A_w_q: jax.Array,
    A_w_uk: jax.Array,
    A_w_uv: jax.Array,
    A_w_o: jax.Array,
    B_x: jax.Array,
    B_w_r: jax.Array,
    B_w_gate: jax.Array,
    B_w_up: jax.Array,
    B_w_down: jax.Array,
):
    del B_x
    return _call(A_x, A_c_kv, A_w_q, A_w_uk, A_w_uv, A_w_o,
                 B_w_r, B_w_gate, B_w_up, B_w_down, _CFG)
```

```python
import functools

import jax
import jax.numpy as jnp
from jax import lax
import jax.experimental.pallas as pl
import jax.experimental.pallas.tpu as pltpu

_F32 = jnp.float32
_BF16 = jnp.bfloat16
_LANES = 128
_NT = (((1,), (1,)), ((), ()))

_REGIONS = 8
_PER_UNIT = 4
_PIECE = 32
_AHEAD = 3
_RING = 4
_ROWS = 16


def _layernorm(x):
    m = jnp.mean(x, axis=-1, keepdims=True)
    d = x - m
    v = jnp.mean(d * d, axis=-1, keepdims=True)
    return d / jnp.sqrt(v + 1e-5)


def _bounds(sizes):
    out, lo = [], 0
    for s in sizes:
        out.append((lo, s))
        lo += s
    return out


def _kernel(
    x_hbm, ckv_hbm, wq_hbm, wuk_hbm, wuv_hbm, wo_hbm, wr_hbm, wg_hbm, wu_hbm, wd_hbm,
    o_ref,
    x_v, wr_v, wq_v, wuk_v, ckv_v, wuv_v, wo_v, wg_v, wu_v, wd_v,
    rows_v, ctx_v, col_v, ring_sems, io_sems, ffn_sems,
    *, cfg,
):
    NU, _, TU, H, D = wq_v.shape
    NKV, TK, Dc = ckv_v.shape
    M = wo_v.shape[2]
    F = wg_hbm.shape[0]
    Fp = wg_v.shape[0]
    J = _LANES // H
    T = Dc // J
    G = cfg["G"]
    order = cfg["order"]

    def slab_piece(w_hbm, w_v):
        n = TU // _PER_UNIT
        return lambda u, r, i: (w_hbm.at[pl.ds(r * (NU * TU) + u * TU + i * n, n)],
                                w_v.at[u, r, pl.ds(i * n, n)])

    def kv_piece(u, r, i):
        row = (r * NKV + u) * (_PER_UNIT * _PIECE) + i * _PIECE
        return (ckv_hbm.at[0, pl.ds(pl.multiple_of(row, _PIECE), _PIECE)],
                ckv_v.at[u, pl.ds((r * _PER_UNIT + i) * _PIECE, _PIECE)])

    def wo_piece(u, r, i):
        return (wo_hbm.at[r * NU + u, pl.ds(i * _PIECE, _PIECE)],
                wo_v.at[u, pl.ds((r * _PER_UNIT + i) * _PIECE, _PIECE)])

    phases = [(slab_piece(wq_hbm, wq_v), wq_v), (slab_piece(wuk_hbm, wuk_v), wuk_v),
              (kv_piece, ckv_v), (slab_piece(wuv_hbm, wuv_v), wuv_v), (wo_piece, wo_v)]
    assert all(buf.shape[0] % _RING == 0 for _, buf in phases)

    def start_unit(p, u):
        for i in range(_PER_UNIT):
            for k, r in enumerate(order):
                src, dst = phases[p][0](u, r, i)
                pltpu.make_async_copy(src, dst, ring_sems.at[u % _RING]).start(priority=k % 2)

    n_pieces = F // _PIECE
    per = cfg["ffn_stride"]
    hidden = [j for i in range(per) for j in range(i, n_pieces, per)]
    gu_units = _bounds(cfg["gu_pieces"])
    wd_units = _bounds(cfg["wd_pieces"])
    ffn_queue, ffn_ends = [], []
    for k, (lo, n) in enumerate(gu_units):
        for i in range(lo, lo + n):
            ffn_queue += [(wg_hbm, wg_v, i, 2 * k), (wu_hbm, wu_v, i, 2 * k + 1)]
        ffn_ends.append(len(ffn_queue))
    for k, (lo, n) in enumerate(wd_units):
        ffn_queue += [(wd_hbm, wd_v, i, 2 * len(gu_units) + k) for i in range(lo, lo + n)]
        ffn_ends.append(len(ffn_queue))
    unit_pieces = _REGIONS * _PER_UNIT

    def start_ffn(lo, hi):
        for k in range(lo, min(hi, len(ffn_queue))):
            src, dst, i, s = ffn_queue[k]
            pltpu.make_async_copy(src.at[pl.ds(hidden[i] * _PIECE, _PIECE)],
                                  dst.at[pl.ds(i * _PIECE, _PIECE)],
                                  ffn_sems.at[s]).start(priority=k % 2)

    def wait_rows(buf, lo, n, sem):
        rows = buf.at[pl.ds(lo * _PIECE, n * _PIECE)]
        pltpu.make_async_copy(rows, rows, sem).wait()

    def advance(p, u):
        buf = phases[p][1]
        n = buf.shape[0]
        pl.when(u + _AHEAD < n)(lambda: start_unit(p, u + _AHEAD))
        if p + 1 < len(phases):
            pl.when(u + _AHEAD >= n)(lambda: start_unit(p + 1, u + _AHEAD - n))
        else:
            for k in range(_AHEAD):
                pl.when(u + _AHEAD == n + k)(
                    functools.partial(start_ffn, k * unit_pieces, (k + 1) * unit_pieces))
        pltpu.make_async_copy(buf.at[u], buf.at[u], ring_sems.at[u % _RING]).wait()

    cp_x = pltpu.make_async_copy(x_hbm, x_v, io_sems.at[0])
    cp_wr = pltpu.make_async_copy(wr_hbm, wr_v, io_sems.at[1])
    cp_x.start(priority=0)
    cp_wr.start(priority=1)
    lax.fori_loop(0, _AHEAD, lambda u, c: start_unit(0, u), None)

    if Fp > F:
        for buf in (wg_v, wu_v):
            buf[F:Fp, :] = jnp.zeros((Fp - F, M), _BF16)

    diag = (lax.broadcasted_iota(jnp.int32, (H, J * H), 1) % H
            == lax.broadcasted_iota(jnp.int32, (H, J * H), 0))
    halves = _REGIONS // J
    per_half = TU // G

    def tile_group(w_v, u, k):
        half, t0 = k // per_half, (k % per_half) * G
        w = jnp.concatenate(
            [w_v[u, halves * j + half, t0 + g] for g in range(G) for j in range(J)], axis=0)
        return w, pl.multiple_of(half * (NU * TU) + u * TU + t0, G)

    def head_contract(p):
        def unit(u, acc):
            advance(p, u)

            def group(k, acc):
                w, t = tile_group(phases[p][1], u, k)
                r = rows_v[pl.ds(t, G), :]
                s = jnp.concatenate(
                    [jnp.where(diag, r[g:g + 1, :], 0.0) for g in range(G)], axis=1)
                return acc + jnp.dot(s.astype(_BF16), w, preferred_element_type=_F32)
            return lax.fori_loop(0, halves * per_half, group, acc)
        return lax.fori_loop(0, NU, unit, jnp.zeros((H, D), _F32))

    cp_x.wait()
    x = x_v[0].astype(_F32)
    xn = _layernorm(x)
    rows_v[...] = jnp.concatenate(
        [jnp.broadcast_to(xn[:, j * T:(j + 1) * T], (H, T)) for j in range(J)], axis=0).T
    q = head_contract(0).astype(_BF16)

    def absorb(u, carry):
        advance(1, u)

        def group(k, carry):
            w, t = tile_group(wuk_v, u, k)
            r = lax.dot_general(q, w, _NT, preferred_element_type=_F32)
            rows_v[pl.ds(t, G), :] = jnp.concatenate(
                [jnp.sum(jnp.where(diag, r[:, g * J * H:(g + 1) * J * H], 0.0),
                         axis=0, keepdims=True) for g in range(G)], axis=0)
            return carry
        return lax.fori_loop(0, halves * per_half, group, carry)
    lax.fori_loop(0, NU, absorb, None)
    qt = rows_v[...].T
    qa = jnp.concatenate([qt[j * H:(j + 1) * H, :] for j in range(J)], axis=1)
    qa = (qa * (D ** -0.5)).astype(_BF16)

    def attend(u, carry):
        m, l, acc = carry
        advance(2, u)
        s = lax.dot_general(qa, ckv_v[u], _NT, preferred_element_type=_F32)
        m_new = jnp.maximum(m, jnp.max(s, axis=-1, keepdims=True))
        alpha = jnp.exp(m - m_new)
        p = jnp.exp(s - m_new)
        l = alpha * l + jnp.sum(p, axis=-1, keepdims=True)
        acc = alpha * acc + jnp.dot(p.astype(_BF16), ckv_v[u], preferred_element_type=_F32)
        return m_new, l, acc

    _, l, acc = lax.fori_loop(
        0, NKV, attend,
        (jnp.full((H, 1), -jnp.inf, _F32), jnp.zeros((H, 1), _F32), jnp.zeros((H, Dc), _F32)))
    lat = acc / l

    rows_v[...] = jnp.concatenate([lat[:, j * T:(j + 1) * T] for j in range(J)], axis=0).T
    ctx_v[...] = head_contract(3)

    def out_proj(u, attn):
        advance(4, u)
        for r in range(_REGIONS):
            a = jnp.broadcast_to(ctx_v[pl.ds(r * NU + u, 1), :], (_ROWS, D)).astype(_BF16)
            attn += jnp.dot(a, wo_v[u, r * D:(r + 1) * D, :], preferred_element_type=_F32)
        return attn
    attn = lax.fori_loop(0, NU, out_proj, jnp.zeros((_ROWS, M), _F32))

    h = x + attn
    hn = _layernorm(h)
    hb = hn.astype(_BF16)

    cp_wr.wait()
    r = jnp.sum(hn * wr_v[...].astype(_F32).reshape(1, M), axis=-1, keepdims=True)
    gate = jax.nn.sigmoid(r)

    queued = _AHEAD * unit_pieces

    def top_up(k):
        nonlocal queued
        target = ffn_ends[k] + _AHEAD * unit_pieces
        start_ffn(queued, target)
        queued = max(queued, target)

    for k, (lo, n) in enumerate(gu_units):
        top_up(k)
        wait_rows(wg_v, lo, n, ffn_sems.at[2 * k])
        wait_rows(wu_v, lo, n, ffn_sems.at[2 * k + 1])
        c0, c1 = lo * _PIECE, pl.cdiv((lo + n) * _PIECE, _LANES) * _LANES
        g = lax.dot_general(hb, wg_v[c0:c1, :], _NT, preferred_element_type=_F32)[0:8]
        up = lax.dot_general(hb, wu_v[c0:c1, :], _NT, preferred_element_type=_F32)[0:8]
        coef = jax.nn.silu(g) * up * gate[0:8]
        for c in range(c0, c1, _LANES):
            col_v[c:c + _LANES, :] = jnp.broadcast_to(
                coef[0:1, c - c0:c - c0 + _LANES], (_LANES, _LANES)).T

    first = lax.broadcasted_iota(jnp.int32, (8, M), 0) == 0
    out = jnp.where(first, (h + (hn + hn * 0.0))[0:8], 0.0)
    out = [out[:, c:c + _LANES] for c in range(0, M, _LANES)]
    for k, (lo, n) in enumerate(wd_units):
        top_up(len(gu_units) + k)
        wait_rows(wd_v, lo, n, ffn_sems.at[2 * len(gu_units) + k])
        for c in range(lo * _PIECE, (lo + n) * _PIECE, 16):
            w = wd_v[c:c + 16, :].astype(_F32)
            a = col_v[c:c + 16, :]
            for j in range(M // _LANES):
                t = w[:, j * _LANES:(j + 1) * _LANES] * a
                out[j] = out[j] + (t[0:8] + t[8:16])
    o_ref[0] = jnp.sum(jnp.concatenate(out, axis=1), axis=0, keepdims=True).astype(o_ref.dtype)


_CFG = dict(
    G=16,
    order=(0, 4, 2, 6, 1, 5, 3, 7),
    ffn_stride=16,
    gu_pieces=(16, 16, 11),
    wd_pieces=(20, 10, 6, 4, 3),
)


def _call(A_x, A_c_kv, A_w_q, A_w_uk, A_w_uv, A_w_o, B_w_r, B_w_gate, B_w_up, B_w_down, cfg):
    B, Sq, M = A_x.shape
    _, Sk, Dc = A_c_kv.shape
    _, H, D = A_w_q.shape
    F = B_w_down.shape[0]
    unit_rows = _REGIONS * _PER_UNIT * _PIECE
    NU = H * D // unit_rows
    assert B == 1 and Sq == 1 and M == Dc and D == _LANES and Dc * H == _LANES * _LANES
    assert D == _PER_UNIT * _PIECE and Sk % (NU * unit_rows) == 0 and F % _PIECE == 0
    Fp = pl.cdiv(F, _LANES) * _LANES
    slabs = (NU, _REGIONS, Dc // (NU * _REGIONS), H, D)
    hbm = pl.BlockSpec(memory_space=pltpu.MemorySpace.HBM)
    return pl.pallas_call(
        functools.partial(_kernel, cfg=cfg),
        in_specs=[hbm] * 10,
        out_specs=pl.BlockSpec(memory_space=pltpu.MemorySpace.VMEM),
        out_shape=jax.ShapeDtypeStruct((B, Sq, M), A_x.dtype),
        scratch_shapes=[
            pltpu.VMEM((B, Sq, M), _BF16),
            pltpu.VMEM((M,), _BF16),
            pltpu.VMEM(slabs, _BF16),
            pltpu.VMEM(slabs, _BF16),
            pltpu.VMEM((Sk // unit_rows, unit_rows, Dc), _BF16),
            pltpu.VMEM(slabs, _BF16),
            pltpu.VMEM((NU, unit_rows, M), _BF16),
            pltpu.VMEM((Fp, M), _BF16),
            pltpu.VMEM((Fp, M), _BF16),
            pltpu.VMEM((F, M), _BF16),
            pltpu.VMEM((_LANES, _LANES), _F32),
            pltpu.VMEM((H, D), _F32),
            pltpu.VMEM((Fp, _LANES), _F32),
            pltpu.SemaphoreType.DMA((_RING,)),
            pltpu.SemaphoreType.DMA((2,)),
            pltpu.SemaphoreType.DMA((2 * len(cfg["gu_pieces"]) + len(cfg["wd_pieces"]),)),
        ],
        compiler_params=pltpu.CompilerParams(
            vmem_limit_bytes=64 * 1024 * 1024,
            disable_semaphore_checks=cfg.get("no_sem_checks", True),
            disable_bounds_checks=cfg.get("no_bounds_checks", True),
        ),
    )(
        A_x, A_c_kv, A_w_q, A_w_uk, A_w_uv, A_w_o, B_w_r,
        B_w_gate.T, B_w_up.T, B_w_down,
    )


@jax.jit
def pallas_sequential_preLN__compressed_kv_cla__moe_arch_mod__decode_kernel(
    A_x: jax.Array,
    A_c_kv: jax.Array,
    A_w_q: jax.Array,
    A_w_uk: jax.Array,
    A_w_uv: jax.Array,
    A_w_o: jax.Array,
    B_x: jax.Array,
    B_w_r: jax.Array,
    B_w_gate: jax.Array,
    B_w_up: jax.Array,
    B_w_down: jax.Array,
):
    del B_x
    return _call(A_x, A_c_kv, A_w_q, A_w_uk, A_w_uv, A_w_o,
                 B_w_r, B_w_gate, B_w_up, B_w_down, _CFG)
```

```python
import functools

import jax
import jax.numpy as jnp
from jax import lax
import jax.experimental.pallas as pl
import jax.experimental.pallas.tpu as pltpu

_F32 = jnp.float32
_BF16 = jnp.bfloat16
_LANES = 128
_NT = (((1,), (1,)), ((), ()))

_REGIONS = 8
_PER_UNIT = 4
_PIECE = 32
_AHEAD = 3
_RING = 4
_ROWS = 16


def _layernorm(x):
    m = jnp.mean(x, axis=-1, keepdims=True)
    d = x - m
    v = jnp.mean(d * d, axis=-1, keepdims=True)
    return d / jnp.sqrt(v + 1e-5)


def _bounds(sizes):
    out, lo = [], 0
    for s in sizes:
        out.append((lo, s))
        lo += s
    return out


def _kernel(
    x_hbm, ckv_hbm, wq_hbm, wuk_hbm, wuv_hbm, wo_hbm, wr_hbm, wg_hbm, wu_hbm, wd_hbm,
    o_ref,
    x_v, wr_v, wq_v, wuk_v, ckv_v, wuv_v, wo_v, wg_v, wu_v, wd_v,
    rows_v, ctx_v, col_v, ring_sems, io_sems, ffn_sems,
    *, cfg,
):
    NU, J, TU, H, D = wq_v.shape
    Dc = ckv_v.shape[2]
    M = wo_v.shape[2]
    F = wg_hbm.shape[0]
    Fp = wg_v.shape[0]
    T = NU * TU
    order = cfg["order"]

    def slab_piece(w_hbm, w_v, u, j, i):
        n = TU // _PER_UNIT
        return w_hbm.at[pl.ds(j * T + u * TU + i * n, n)], w_v.at[u, j, pl.ds(i * n, n)]

    def wo_piece(u, j, i):
        return (wo_hbm.at[j * NU + u, pl.ds(i * _PIECE, _PIECE)],
                wo_v.at[u, pl.ds(j * D + i * _PIECE, _PIECE)])

    def kv_piece(u, r, i):
        row = (r * NU + u) * (_PER_UNIT * _PIECE) + i * _PIECE
        return (ckv_hbm.at[0, pl.ds(pl.multiple_of(row, _PIECE), _PIECE)],
                ckv_v.at[u, pl.ds((r * _PER_UNIT + i) * _PIECE, _PIECE)])

    phases = [
        [(functools.partial(slab_piece, wq_hbm, wq_v), wq_v),
         (functools.partial(slab_piece, wuk_hbm, wuk_v), wuk_v)],
        [(kv_piece, ckv_v)],
        [(functools.partial(slab_piece, wuv_hbm, wuv_v), wuv_v), (wo_piece, wo_v)],
    ]
    n_units = len(phases) * NU
    assert NU % _RING == 0 and _AHEAD < _RING

    def start_unit(p, u):
        per_array = _REGIONS // len(phases[p])
        for i in range(_PER_UNIT):
            for k, r in enumerate(order):
                a = r // per_array
                src, dst = phases[p][a][0](u, r % per_array, i)
                pltpu.make_async_copy(
                    src, dst, ring_sems.at[a * _RING + u % _RING]).start(priority=k % 2)

    def wait_unit(p, u):
        for a, (_, buf) in enumerate(phases[p]):
            pltpu.make_async_copy(
                buf.at[u], buf.at[u], ring_sems.at[a * _RING + u % _RING]).wait()

    n_pieces = F // _PIECE
    per = cfg["ffn_stride"]
    hidden = [j for i in range(per) for j in range(i, n_pieces, per)]
    gu_units = _bounds(cfg["gu_pieces"])
    wd_units = _bounds(cfg["wd_pieces"])
    ffn_queue, ffn_ends = [], []
    for k, (lo, n) in enumerate(gu_units):
        for i in range(lo, lo + n):
            ffn_queue += [(wg_hbm, wg_v, i, 2 * k), (wu_hbm, wu_v, i, 2 * k + 1)]
        ffn_ends.append(len(ffn_queue))
    for k, (lo, n) in enumerate(wd_units):
        ffn_queue += [(wd_hbm, wd_v, i, 2 * len(gu_units) + k) for i in range(lo, lo + n)]
        ffn_ends.append(len(ffn_queue))
    unit_pieces = _REGIONS * _PER_UNIT

    def start_ffn(lo, hi):
        for k in range(lo, min(hi, len(ffn_queue))):
            src, dst, i, s = ffn_queue[k]
            pltpu.make_async_copy(src.at[pl.ds(hidden[i] * _PIECE, _PIECE)],
                                  dst.at[pl.ds(i * _PIECE, _PIECE)],
                                  ffn_sems.at[s]).start(priority=k % 2)

    def wait_rows(buf, lo, n, sem):
        rows = buf.at[pl.ds(lo * _PIECE, n * _PIECE)]
        pltpu.make_async_copy(rows, rows, sem).wait()

    def for_unit(fn, n, lo, hi):
        for p in range(lo // NU, pl.cdiv(min(hi, n_units), NU)):
            if p * NU <= lo and hi <= (p + 1) * NU:
                fn(p, n - p * NU)
            else:
                pl.when((n >= p * NU) & (n < (p + 1) * NU))(
                    lambda p=p: fn(p, n - p * NU))

    def follow_stream(lo, hi, body, init):
        def step(n, carry):
            for_unit(start_unit, n + _AHEAD, lo + _AHEAD, hi + _AHEAD)
            for k in range(max(0, hi + _AHEAD - n_units)):
                pl.when(n + _AHEAD == n_units + k)(
                    functools.partial(start_ffn, k * unit_pieces, (k + 1) * unit_pieces))
            for_unit(wait_unit, n, lo, hi)
            return body(n - lo, carry)
        return lax.fori_loop(lo, hi, step, init)

    cp_x = pltpu.make_async_copy(x_hbm, x_v, io_sems.at[0])
    cp_wr = pltpu.make_async_copy(wr_hbm, wr_v, io_sems.at[1])
    cp_x.start(priority=0)
    cp_wr.start(priority=1)
    lax.fori_loop(0, _AHEAD, lambda u, c: start_unit(0, u), None)

    if Fp > F:
        for buf in (wg_v, wu_v):
            buf[F:Fp, :] = jnp.zeros((Fp - F, M), _BF16)

    diag = (lax.broadcasted_iota(jnp.int32, (H, J * H), 1) % H
            == lax.broadcasted_iota(jnp.int32, (H, J * H), 0))

    def tiles(w_v, u):
        return jnp.concatenate([w_v[u, j, t] for t in range(TU) for j in range(J)], axis=0)

    def head_contract(w_v, u, acc):
        r = rows_v[pl.ds(pl.multiple_of(u * TU, TU), TU), :]
        s = jnp.concatenate(
            [jnp.where(diag, r[t:t + 1, :], 0.0) for t in range(TU)], axis=1)
        return acc + jnp.dot(s.astype(_BF16), tiles(w_v, u), preferred_element_type=_F32)

    cp_x.wait()
    x = x_v[0].astype(_F32)
    xn = _layernorm(x)
    rows_v[...] = jnp.concatenate(
        [jnp.broadcast_to(xn[:, j * T:(j + 1) * T], (H, T)) for j in range(J)], axis=0).T
    q = follow_stream(0, NU, functools.partial(head_contract, wq_v), jnp.zeros((H, D), _F32))
    q = q.astype(_BF16)

    def absorb(u, carry):
        r = lax.dot_general(q, tiles(wuk_v, u), _NT, preferred_element_type=_F32)
        rows_v[pl.ds(pl.multiple_of(u * TU, TU), TU), :] = jnp.concatenate(
            [jnp.sum(jnp.where(diag, r[:, t * J * H:(t + 1) * J * H], 0.0),
                     axis=0, keepdims=True) for t in range(TU)], axis=0)
        return carry
    lag = NU // 2
    follow_stream(NU, NU + lag, lambda k, c: lax.fori_loop(2 * k, 2 * k + 2, absorb, c), None)
    qt = rows_v[...].T
    qa = jnp.concatenate([qt[j * H:(j + 1) * H, :] for j in range(J)], axis=1)
    qa = (qa * (D ** -0.5)).astype(_BF16)

    def attend(u, carry):
        m, l, acc = carry
        s = lax.dot_general(qa, ckv_v[u], _NT, preferred_element_type=_F32)
        m_new = jnp.maximum(m, jnp.max(s, axis=-1, keepdims=True))
        alpha = jnp.exp(m - m_new)
        p = jnp.exp(s - m_new)
        l = alpha * l + jnp.sum(p, axis=-1, keepdims=True)
        acc = alpha * acc + jnp.dot(p.astype(_BF16), ckv_v[u], preferred_element_type=_F32)
        return m_new, l, acc

    _, l, acc = follow_stream(
        NU + lag, 2 * NU + lag, attend,
        (jnp.full((H, 1), -jnp.inf, _F32), jnp.zeros((H, 1), _F32), jnp.zeros((H, Dc), _F32)))
    lat = acc / l

    rows_v[...] = jnp.concatenate([lat[:, j * T:(j + 1) * T] for j in range(J)], axis=0).T
    contract = functools.partial(head_contract, wuv_v)
    ctx_v[...] = follow_stream(
        2 * NU + lag, 3 * NU,
        lambda k, c: lax.fori_loop(jnp.where(k == 0, 0, lag + k), lag + k + 1, contract, c),
        jnp.zeros((H, D), _F32))

    def out_proj(u, attn):
        for j in range(J):
            a = jnp.broadcast_to(ctx_v[pl.ds(j * NU + u, 1), :], (_ROWS, D)).astype(_BF16)
            attn += jnp.dot(a, wo_v[u, j * D:(j + 1) * D, :], preferred_element_type=_F32)
        return attn
    attn = lax.fori_loop(0, NU, out_proj, jnp.zeros((_ROWS, M), _F32), unroll=cfg["wo_unroll"])

    h = x + attn
    hn = _layernorm(h)
    hb = hn.astype(_BF16)

    cp_wr.wait()
    r = jnp.sum(hn * wr_v[...].astype(_F32).reshape(1, M), axis=-1, keepdims=True)
    gate = jax.nn.sigmoid(r)

    queued = _AHEAD * unit_pieces

    def top_up(k):
        nonlocal queued
        target = ffn_ends[k] + _AHEAD * unit_pieces
        start_ffn(queued, target)
        queued = max(queued, target)

    for k, (lo, n) in enumerate(gu_units):
        top_up(k)
        wait_rows(wg_v, lo, n, ffn_sems.at[2 * k])
        wait_rows(wu_v, lo, n, ffn_sems.at[2 * k + 1])
        c0, c1 = lo * _PIECE, pl.cdiv((lo + n) * _PIECE, _LANES) * _LANES
        g = lax.dot_general(hb, wg_v[c0:c1, :], _NT, preferred_element_type=_F32)[0:8]
        up = lax.dot_general(hb, wu_v[c0:c1, :], _NT, preferred_element_type=_F32)[0:8]
        coef = jax.nn.silu(g) * up * gate[0:8]
        for c in range(c0, c1, _LANES):
            col_v[c:c + _LANES, :] = jnp.broadcast_to(
                coef[0:1, c - c0:c - c0 + _LANES], (_LANES, _LANES)).T

    first = lax.broadcasted_iota(jnp.int32, (8, M), 0) == 0
    out = jnp.where(first, (h + (hn + hn * 0.0))[0:8], 0.0)
    out = [out[:, c:c + _LANES] for c in range(0, M, _LANES)]
    for k, (lo, n) in enumerate(wd_units):
        top_up(len(gu_units) + k)
        wait_rows(wd_v, lo, n, ffn_sems.at[2 * len(gu_units) + k])
        for c in range(lo * _PIECE, (lo + n) * _PIECE, 16):
            w = wd_v[c:c + 16, :].astype(_F32)
            a = col_v[c:c + 16, :]
            for j in range(M // _LANES):
                t = w[:, j * _LANES:(j + 1) * _LANES] * a
                out[j] = out[j] + (t[0:8] + t[8:16])
    o_ref[0] = jnp.sum(jnp.concatenate(out, axis=1), axis=0, keepdims=True).astype(o_ref.dtype)


_CFG = dict(
    wo_unroll=2,
    order=(0, 1, 2, 3, 4, 5, 6, 7),
    ffn_stride=16,
    gu_pieces=(16, 16, 11),
    wd_pieces=(20, 10, 6, 4, 3),
)


def _call(A_x, A_c_kv, A_w_q, A_w_uk, A_w_uv, A_w_o, B_w_r, B_w_gate, B_w_up, B_w_down, cfg):
    B, Sq, M = A_x.shape
    _, Sk, Dc = A_c_kv.shape
    _, H, D = A_w_q.shape
    F = B_w_down.shape[0]
    unit_rows = _REGIONS * _PER_UNIT * _PIECE
    NU = Sk // unit_rows
    J = _REGIONS // 2
    assert B == 1 and Sq == 1 and M == Dc and D == _LANES and J * H == _LANES
    assert D == _PER_UNIT * _PIECE and J * NU == H and Dc == J * _LANES
    assert Sk == NU * unit_rows and F % _PIECE == 0
    Fp = pl.cdiv(F, _LANES) * _LANES
    slabs = (NU, J, _LANES // NU, H, D)
    hbm = pl.BlockSpec(memory_space=pltpu.MemorySpace.HBM)
    return pl.pallas_call(
        functools.partial(_kernel, cfg=cfg),
        in_specs=[hbm] * 10,
        out_specs=pl.BlockSpec(memory_space=pltpu.MemorySpace.VMEM),
        out_shape=jax.ShapeDtypeStruct((B, Sq, M), A_x.dtype),
        scratch_shapes=[
            pltpu.VMEM((B, Sq, M), _BF16),
            pltpu.VMEM((M,), _BF16),
            pltpu.VMEM(slabs, _BF16),
            pltpu.VMEM(slabs, _BF16),
            pltpu.VMEM((NU, unit_rows, Dc), _BF16),
            pltpu.VMEM(slabs, _BF16),
            pltpu.VMEM((NU, J * D, M), _BF16),
            pltpu.VMEM((Fp, M), _BF16),
            pltpu.VMEM((Fp, M), _BF16),
            pltpu.VMEM((F, M), _BF16),
            pltpu.VMEM((_LANES, _LANES), _F32),
            pltpu.VMEM((H, D), _F32),
            pltpu.VMEM((Fp, _LANES), _F32),
            pltpu.SemaphoreType.DMA((2 * _RING,)),
            pltpu.SemaphoreType.DMA((2,)),
            pltpu.SemaphoreType.DMA((2 * len(cfg["gu_pieces"]) + len(cfg["wd_pieces"]),)),
        ],
        compiler_params=pltpu.CompilerParams(
            vmem_limit_bytes=64 * 1024 * 1024,
            disable_semaphore_checks=cfg.get("no_sem_checks", True),
            disable_bounds_checks=cfg.get("no_bounds_checks", True),
        ),
    )(
        A_x, A_c_kv, A_w_q, A_w_uk, A_w_uv, A_w_o, B_w_r,
        B_w_gate.T, B_w_up.T, B_w_down,
    )


@jax.jit
def pallas_sequential_preLN__compressed_kv_cla__moe_arch_mod__decode_kernel(
    A_x: jax.Array,
    A_c_kv: jax.Array,
    A_w_q: jax.Array,
    A_w_uk: jax.Array,
    A_w_uv: jax.Array,
    A_w_o: jax.Array,
    B_x: jax.Array,
    B_w_r: jax.Array,
    B_w_gate: jax.Array,
    B_w_up: jax.Array,
    B_w_down: jax.Array,
):
    del B_x
    return _call(A_x, A_c_kv, A_w_q, A_w_uk, A_w_uv, A_w_o,
                 B_w_r, B_w_gate, B_w_up, B_w_down, _CFG)
```

```python
import functools

import jax
import jax.numpy as jnp
from jax import lax
import jax.experimental.pallas as pl
import jax.experimental.pallas.tpu as pltpu

_F32 = jnp.float32
_BF16 = jnp.bfloat16
_LANES = 128
_NT = (((1,), (1,)), ((), ()))

_REGIONS = 8
_PER_UNIT = 4
_PIECE = 32
_AHEAD = 3
_RING = 4
_ROWS = 16


def _layernorm(x):
    m = jnp.mean(x, axis=-1, keepdims=True)
    d = x - m
    v = jnp.mean(d * d, axis=-1, keepdims=True)
    return d / jnp.sqrt(v + 1e-5)


def _bounds(sizes):
    out, lo = [], 0
    for s in sizes:
        out.append((lo, s))
        lo += s
    return out


def _kernel(
    x_hbm, ckv_hbm, wq_hbm, wuk_hbm, wuv_hbm, wo_hbm, wr_hbm, wg_hbm, wu_hbm, wd_hbm,
    o_ref,
    x_v, wr_v, wq_v, wuk_v, ckv_v, wuv_v, wo_v, wg_v, wu_v, wd_v,
    rows_v, ctx_v, col_v, ring_sems, io_sems, ffn_sems,
    *, cfg,
):
    NU, J, TU, H, D = wq_v.shape
    Dc = ckv_v.shape[2]
    M = wo_v.shape[2]
    F = wg_hbm.shape[0]
    T = NU * TU
    order = cfg["order"]

    def slab_piece(w_hbm, w_v, u, j, i):
        n = TU // _PER_UNIT
        return w_hbm.at[pl.ds(j * T + u * TU + i * n, n)], w_v.at[u, j, pl.ds(i * n, n)]

    def wo_piece(u, j, i):
        return (wo_hbm.at[j * NU + u, pl.ds(i * _PIECE, _PIECE)],
                wo_v.at[u, pl.ds(j * D + i * _PIECE, _PIECE)])

    def kv_piece(u, r, i):
        row = (r * NU + u) * (_PER_UNIT * _PIECE) + i * _PIECE
        return (ckv_hbm.at[0, pl.ds(pl.multiple_of(row, _PIECE), _PIECE)],
                ckv_v.at[u, pl.ds((r * _PER_UNIT + i) * _PIECE, _PIECE)])

    phases = [
        [(functools.partial(slab_piece, wq_hbm, wq_v), wq_v),
         (functools.partial(slab_piece, wuk_hbm, wuk_v), wuk_v)],
        [(kv_piece, ckv_v)],
        [(functools.partial(slab_piece, wuv_hbm, wuv_v), wuv_v), (wo_piece, wo_v)],
    ]
    n_units = len(phases) * NU
    assert NU % _RING == 0 and _AHEAD < _RING

    def start_unit(p, u):
        per_array = _REGIONS // len(phases[p])
        for i in range(_PER_UNIT):
            for k, r in enumerate(order):
                a = r // per_array
                src, dst = phases[p][a][0](u, r % per_array, i)
                pltpu.make_async_copy(
                    src, dst, ring_sems.at[a * _RING + u % _RING]).start(priority=k % 2)

    def wait_unit(p, u):
        for a, (_, buf) in enumerate(phases[p]):
            pltpu.make_async_copy(
                buf.at[u], buf.at[u], ring_sems.at[a * _RING + u % _RING]).wait()

    n_pieces = F // _PIECE

    def strided(stride):
        return [j for i in range(stride) for j in range(i, n_pieces, stride)]
    gu_order, wd_order = strided(cfg["gu_stride"]), strided(cfg["wd_stride"])
    gu_units, wd_units = _bounds(cfg["gu_pieces"]), _bounds(cfg["wd_pieces"])
    ffn_queue, ffn_ends = [], []
    group = cfg["gu_group"]
    for k, (lo, n) in enumerate(gu_units):
        for i0 in range(lo, lo + n, group):
            for a, (src, dst) in enumerate([(wg_hbm, wg_v), (wu_hbm, wu_v)]):
                ffn_queue += [(src, dst, gu_order[i], i, 2 * k + a)
                              for i in range(i0, min(i0 + group, lo + n))]
        ffn_ends.append(len(ffn_queue))
    for k, (lo, n) in enumerate(wd_units):
        ffn_queue += [(wd_hbm, wd_v, wd_order[i], i, 2 * len(gu_units) + k)
                      for i in range(lo, lo + n)]
        ffn_ends.append(len(ffn_queue))
    unit_pieces = _REGIONS * _PER_UNIT

    def start_ffn(lo, hi):
        for k in range(lo, min(hi, len(ffn_queue))):
            src, dst, piece, i, s = ffn_queue[k]
            pltpu.make_async_copy(src.at[pl.ds(piece * _PIECE, _PIECE)],
                                  dst.at[pl.ds(i * _PIECE, _PIECE)],
                                  ffn_sems.at[s]).start(priority=k % 2)

    def wait_rows(buf, lo, n, sem):
        rows = buf.at[pl.ds(lo * _PIECE, n * _PIECE)]
        pltpu.make_async_copy(rows, rows, sem).wait()

    def for_unit(fn, n, lo, hi):
        for p in range(lo // NU, pl.cdiv(min(hi, n_units), NU)):
            if p * NU <= lo and hi <= (p + 1) * NU:
                fn(p, n - p * NU)
            else:
                pl.when((n >= p * NU) & (n < (p + 1) * NU))(
                    lambda p=p: fn(p, n - p * NU))

    def follow_stream(lo, hi, body, init):
        def step(n, carry):
            for_unit(start_unit, n + _AHEAD, lo + _AHEAD, hi + _AHEAD)
            for k in range(max(0, hi + _AHEAD - n_units)):
                pl.when(n + _AHEAD == n_units + k)(
                    functools.partial(start_ffn, k * unit_pieces, (k + 1) * unit_pieces))
            for_unit(wait_unit, n, lo, hi)
            return body(n - lo, carry)
        return lax.fori_loop(lo, hi, step, init)

    cp_x = pltpu.make_async_copy(x_hbm, x_v, io_sems.at[0])
    cp_wr = pltpu.make_async_copy(wr_hbm, wr_v, io_sems.at[1])
    cp_x.start(priority=0)
    cp_wr.start(priority=1)
    lax.fori_loop(0, _AHEAD, lambda u, c: start_unit(0, u), None)

    diag = (lax.broadcasted_iota(jnp.int32, (H, J * H), 1) % H
            == lax.broadcasted_iota(jnp.int32, (H, J * H), 0))

    def tiles(w_v, u):
        return jnp.concatenate([w_v[u, j, t] for t in range(TU) for j in range(J)], axis=0)

    def head_contract(w_v, u, acc):
        r = rows_v[pl.ds(pl.multiple_of(u * TU, TU), TU), :]
        s = jnp.concatenate(
            [jnp.where(diag, r[t:t + 1, :], 0.0) for t in range(TU)], axis=1)
        return acc + jnp.dot(s.astype(_BF16), tiles(w_v, u), preferred_element_type=_F32)

    cp_x.wait()
    x = x_v[0].astype(_F32)
    xn = _layernorm(x)
    rows_v[...] = jnp.concatenate(
        [jnp.broadcast_to(xn[:, j * T:(j + 1) * T], (H, T)) for j in range(J)], axis=0).T
    q = follow_stream(0, NU, functools.partial(head_contract, wq_v), jnp.zeros((H, D), _F32))
    q = q.astype(_BF16)

    def absorb(u, carry):
        r = lax.dot_general(q, tiles(wuk_v, u), _NT, preferred_element_type=_F32)
        rows_v[pl.ds(pl.multiple_of(u * TU, TU), TU), :] = jnp.concatenate(
            [jnp.sum(jnp.where(diag, r[:, t * J * H:(t + 1) * J * H], 0.0),
                     axis=0, keepdims=True) for t in range(TU)], axis=0)
        return carry
    lag = NU // 2
    follow_stream(NU, NU + lag, lambda k, c: lax.fori_loop(2 * k, 2 * k + 2, absorb, c), None)
    qt = rows_v[...].T
    qa = jnp.concatenate([qt[j * H:(j + 1) * H, :] for j in range(J)], axis=1)
    qa = (qa * (D ** -0.5)).astype(_BF16)

    def attend(u, carry):
        m, l, acc = carry
        s = lax.dot_general(qa, ckv_v[u], _NT, preferred_element_type=_F32)
        m_new = jnp.maximum(m, jnp.max(s, axis=-1, keepdims=True))
        alpha = jnp.exp(m - m_new)
        p = jnp.exp(s - m_new)
        l = alpha * l + jnp.sum(p, axis=-1, keepdims=True)
        acc = alpha * acc + jnp.dot(p.astype(_BF16), ckv_v[u], preferred_element_type=_F32)
        return m_new, l, acc

    _, l, acc = follow_stream(
        NU + lag, 2 * NU + lag, attend,
        (jnp.full((H, 1), -jnp.inf, _F32), jnp.zeros((H, 1), _F32), jnp.zeros((H, Dc), _F32)))
    lat = acc / l

    rows_v[...] = jnp.concatenate([lat[:, j * T:(j + 1) * T] for j in range(J)], axis=0).T
    contract = functools.partial(head_contract, wuv_v)
    ctx_v[...] = follow_stream(
        2 * NU + lag, 3 * NU,
        lambda k, c: lax.fori_loop(jnp.where(k == 0, 0, lag + k), lag + k + 1, contract, c),
        jnp.zeros((H, D), _F32))

    def out_proj(u, attn):
        for j in range(J):
            a = jnp.broadcast_to(ctx_v[pl.ds(j * NU + u, 1), :], (_ROWS, D)).astype(_BF16)
            attn += jnp.dot(a, wo_v[u, j * D:(j + 1) * D, :], preferred_element_type=_F32)
        return attn
    attn = lax.fori_loop(0, NU, out_proj, jnp.zeros((_ROWS, M), _F32), unroll=cfg["wo_unroll"])

    h = x + attn
    hn = _layernorm(h)

    cp_wr.wait()
    r = jnp.sum(hn[0:1] * wr_v[...].astype(_F32).reshape(1, M), axis=-1, keepdims=True)
    gate = jax.nn.sigmoid(r)

    queued = _AHEAD * unit_pieces

    def top_up(k):
        nonlocal queued
        target = ffn_ends[k] + _AHEAD * unit_pieces
        start_ffn(queued, target)
        queued = max(queued, target)

    for k, (lo, n) in enumerate(gu_units):
        top_up(k)
        wait_rows(wg_v, lo, n, ffn_sems.at[2 * k])
        wait_rows(wu_v, lo, n, ffn_sems.at[2 * k + 1])
        for c in range(lo * _PIECE, (lo + n) * _PIECE, cfg["gu_rows"]):
            rows = slice(c, min(c + cfg["gu_rows"], (lo + n) * _PIECE))
            g = jnp.sum(wg_v[rows, :].astype(_F32) * hn[0:1], axis=-1, keepdims=True)
            up = jnp.sum(wu_v[rows, :].astype(_F32) * hn[0:1], axis=-1, keepdims=True)
            col_v[rows, :] = jnp.broadcast_to(
                jax.nn.silu(g) * up * gate, (rows.stop - rows.start, _LANES))

    first = lax.broadcasted_iota(jnp.int32, (8, M), 0) == 0
    out = jnp.where(first, (h + (hn + hn * 0.0))[0:8], 0.0)
    out = [out[:, c:c + _LANES] for c in range(0, M, _LANES)]
    for k, (lo, n) in enumerate(wd_units):
        top_up(len(gu_units) + k)
        wait_rows(wd_v, lo, n, ffn_sems.at[2 * len(gu_units) + k])
        for c in range(lo * _PIECE, (lo + n) * _PIECE, 16):
            f = gu_order.index(wd_order[c // _PIECE]) * _PIECE + c % _PIECE
            w = wd_v[c:c + 16, :].astype(_F32)
            a = col_v[f:f + 16, :]
            for j in range(M // _LANES):
                t = w[:, j * _LANES:(j + 1) * _LANES] * a
                out[j] = out[j] + (t[0:8] + t[8:16])
    o_ref[0] = jnp.sum(jnp.concatenate(out, axis=1), axis=0, keepdims=True).astype(o_ref.dtype)


_CFG = dict(
    wo_unroll=2,
    order=(0, 1, 2, 3, 4, 5, 6, 7),
    gu_stride=15,
    gu_rows=128,
    wd_stride=8,
    gu_group=1,
    gu_pieces=(16, 16, 11),
    wd_pieces=(20, 10, 6, 4, 3),
)


def _call(A_x, A_c_kv, A_w_q, A_w_uk, A_w_uv, A_w_o, B_w_r, B_w_gate, B_w_up, B_w_down, cfg):
    B, Sq, M = A_x.shape
    _, Sk, Dc = A_c_kv.shape
    _, H, D = A_w_q.shape
    F = B_w_down.shape[0]
    unit_rows = _REGIONS * _PER_UNIT * _PIECE
    NU = Sk // unit_rows
    J = _REGIONS // 2
    assert B == 1 and Sq == 1 and M == Dc and D == _LANES and J * H == _LANES
    assert D == _PER_UNIT * _PIECE and J * NU == H and Dc == J * _LANES
    assert Sk == NU * unit_rows and F % _PIECE == 0
    slabs = (NU, J, _LANES // NU, H, D)
    hbm = pl.BlockSpec(memory_space=pltpu.MemorySpace.HBM)
    return pl.pallas_call(
        functools.partial(_kernel, cfg=cfg),
        in_specs=[hbm] * 10,
        out_specs=pl.BlockSpec(memory_space=pltpu.MemorySpace.VMEM),
        out_shape=jax.ShapeDtypeStruct((B, Sq, M), A_x.dtype),
        scratch_shapes=[
            pltpu.VMEM((B, Sq, M), _BF16),
            pltpu.VMEM((M,), _BF16),
            pltpu.VMEM(slabs, _BF16),
            pltpu.VMEM(slabs, _BF16),
            pltpu.VMEM((NU, unit_rows, Dc), _BF16),
            pltpu.VMEM(slabs, _BF16),
            pltpu.VMEM((NU, J * D, M), _BF16),
            pltpu.VMEM((F, M), _BF16),
            pltpu.VMEM((F, M), _BF16),
            pltpu.VMEM((F, M), _BF16),
            pltpu.VMEM((_LANES, _LANES), _F32),
            pltpu.VMEM((H, D), _F32),
            pltpu.VMEM((F, _LANES), _F32),
            pltpu.SemaphoreType.DMA((2 * _RING,)),
            pltpu.SemaphoreType.DMA((2,)),
            pltpu.SemaphoreType.DMA((2 * len(cfg["gu_pieces"]) + len(cfg["wd_pieces"]),)),
        ],
        compiler_params=pltpu.CompilerParams(
            vmem_limit_bytes=64 * 1024 * 1024,
            disable_semaphore_checks=cfg.get("no_sem_checks", True),
            disable_bounds_checks=cfg.get("no_bounds_checks", True),
        ),
    )(
        A_x, A_c_kv, A_w_q, A_w_uk, A_w_uv, A_w_o, B_w_r,
        B_w_gate.T, B_w_up.T, B_w_down,
    )


@jax.jit
def pallas_sequential_preLN__compressed_kv_cla__moe_arch_mod__decode_kernel(
    A_x: jax.Array,
    A_c_kv: jax.Array,
    A_w_q: jax.Array,
    A_w_uk: jax.Array,
    A_w_uv: jax.Array,
    A_w_o: jax.Array,
    B_x: jax.Array,
    B_w_r: jax.Array,
    B_w_gate: jax.Array,
    B_w_up: jax.Array,
    B_w_down: jax.Array,
):
    del B_x
    return _call(A_x, A_c_kv, A_w_q, A_w_uk, A_w_uv, A_w_o,
                 B_w_r, B_w_gate, B_w_up, B_w_down, _CFG)
```

```python
import functools

import jax
import jax.numpy as jnp
from jax import lax
import jax.experimental.pallas as pl
import jax.experimental.pallas.tpu as pltpu

_F32 = jnp.float32
_BF16 = jnp.bfloat16
_LANES = 128
_NT = (((1,), (1,)), ((), ()))

_PIECE = 32
_REGIONS = 8
_PER_REGION = 4
_UNIT = _REGIONS * _PER_REGION
_AHEAD = 3
_RING = 4
_ROWS = 16

_GU_STRIDE, _GU_UNITS = 16, (16, 16, 11)
_WD_STRIDE, _WD_UNITS = 8, (20, 10, 6, 4, 3)


def _layernorm(x):
    m = jnp.mean(x, axis=-1, keepdims=True)
    d = x - m
    v = jnp.mean(d * d, axis=-1, keepdims=True)
    return d / jnp.sqrt(v + 1e-5)


def _bounds(sizes):
    out, lo = [], 0
    for s in sizes:
        out.append((lo, lo + s))
        lo += s
    return out


def _kernel(
    x_hbm, ckv_hbm, wq_hbm, wuk_hbm, wuv_hbm, wo_hbm, wr_hbm, wg_hbm, wu_hbm, wd_hbm,
    o_ref,
    x_v, wr_v, wq_v, wuk_v, ckv_v, wuv_v, wo_v, wg_v, wu_v, wd_v,
    rows_v, ctx_v, col_v, ring_sems, io_sems, ffn_sems,
):
    NU, J, TU, H, D = wq_v.shape
    Dc = ckv_v.shape[2]
    F, M = wd_v.shape
    T = NU * TU

    def slab_piece(w_hbm, w_v, u, j, i):
        n = TU // _PER_REGION
        return w_hbm.at[pl.ds(j * T + u * TU + i * n, n)], w_v.at[u, j, pl.ds(i * n, n)]

    def wo_piece(u, j, i):
        return (wo_hbm.at[j * NU + u, pl.ds(i * _PIECE, _PIECE)],
                wo_v.at[u, pl.ds(j * D + i * _PIECE, _PIECE)])

    def kv_piece(u, r, i):
        row = ((r * NU + u) * _PER_REGION + i) * _PIECE
        return (ckv_hbm.at[0, pl.ds(pl.multiple_of(row, _PIECE), _PIECE)],
                ckv_v.at[u, pl.ds((r * _PER_REGION + i) * _PIECE, _PIECE)])

    phases = [
        [(functools.partial(slab_piece, wq_hbm, wq_v), wq_v),
         (functools.partial(slab_piece, wuk_hbm, wuk_v), wuk_v)],
        [(kv_piece, ckv_v)],
        [(functools.partial(slab_piece, wuv_hbm, wuv_v), wuv_v), (wo_piece, wo_v)],
    ]
    n_units = len(phases) * NU

    def start_unit(p, u):
        per_array = _REGIONS // len(phases[p])
        for i in range(_PER_REGION):
            for r in range(_REGIONS):
                a = r // per_array
                src, dst = phases[p][a][0](u, r % per_array, i)
                pltpu.make_async_copy(
                    src, dst, ring_sems.at[a * _RING + u % _RING]).start(priority=r % 2)

    def wait_unit(p, u):
        for a, (_, buf) in enumerate(phases[p]):
            pltpu.make_async_copy(
                buf.at[u], buf.at[u], ring_sems.at[a * _RING + u % _RING]).wait()

    def strided(stride):
        return [j for i in range(stride) for j in range(i, F // _PIECE, stride)]

    gu_order, wd_order = strided(_GU_STRIDE), strided(_WD_STRIDE)
    gu_units, wd_units = _bounds(_GU_UNITS), _bounds(_WD_UNITS)
    ffn_queue = []
    for k, (lo, hi) in enumerate(gu_units):
        for i in range(lo, hi):
            ffn_queue += [(wg_hbm, wg_v, gu_order[i], i, 2 * k),
                          (wu_hbm, wu_v, gu_order[i], i, 2 * k + 1)]
    for k, (lo, hi) in enumerate(wd_units):
        ffn_queue += [(wd_hbm, wd_v, wd_order[i], i, 2 * len(gu_units) + k)
                      for i in range(lo, hi)]

    def start_ffn(lo, hi):
        for k in range(lo, hi):
            src, dst, piece, i, s = ffn_queue[k]
            pltpu.make_async_copy(src.at[pl.ds(piece * _PIECE, _PIECE)],
                                  dst.at[pl.ds(i * _PIECE, _PIECE)],
                                  ffn_sems.at[s]).start(priority=k % 2)

    def wait_ffn(buf, lo, hi, s):
        rows = buf.at[pl.ds(lo * _PIECE, (hi - lo) * _PIECE)]
        pltpu.make_async_copy(rows, rows, ffn_sems.at[s]).wait()

    def for_unit(fn, n, lo, hi):
        for p in range(lo // NU, pl.cdiv(min(hi, n_units), NU)):
            if p * NU <= lo and hi <= (p + 1) * NU:
                fn(p, n - p * NU)
            else:
                pl.when((n >= p * NU) & (n < (p + 1) * NU))(
                    lambda p=p: fn(p, n - p * NU))

    def follow_stream(lo, hi, body, init):
        def step(n, carry):
            for_unit(start_unit, n + _AHEAD, lo + _AHEAD, hi + _AHEAD)
            for k in range(max(0, hi + _AHEAD - n_units)):
                pl.when(n + _AHEAD == n_units + k)(
                    functools.partial(start_ffn, k * _UNIT, (k + 1) * _UNIT))
            for_unit(wait_unit, n, lo, hi)
            return body(n - lo, carry)
        return lax.fori_loop(lo, hi, step, init)

    cp_x = pltpu.make_async_copy(x_hbm, x_v, io_sems.at[0])
    cp_wr = pltpu.make_async_copy(wr_hbm, wr_v, io_sems.at[1])
    cp_x.start(priority=0)
    cp_wr.start(priority=1)
    lax.fori_loop(0, _AHEAD, lambda u, c: start_unit(0, u), None)

    diag = (lax.broadcasted_iota(jnp.int32, (H, J * H), 1) % H
            == lax.broadcasted_iota(jnp.int32, (H, J * H), 0))

    def tiles(w_v, u):
        return jnp.concatenate([w_v[u, j, t] for t in range(TU) for j in range(J)], axis=0)

    def head_contract(w_v, u, acc):
        r = rows_v[pl.ds(pl.multiple_of(u * TU, TU), TU), :]
        s = jnp.concatenate(
            [jnp.where(diag, r[t:t + 1, :], 0.0) for t in range(TU)], axis=1)
        return acc + jnp.dot(s.astype(_BF16), tiles(w_v, u), preferred_element_type=_F32)

    cp_x.wait()
    x = x_v[0].astype(_F32)
    xn = _layernorm(x)
    rows_v[...] = jnp.concatenate(
        [jnp.broadcast_to(xn[:, j * T:(j + 1) * T], (H, T)) for j in range(J)], axis=0).T
    q = follow_stream(0, NU, functools.partial(head_contract, wq_v), jnp.zeros((H, D), _F32))
    q = q.astype(_BF16)

    def absorb(u, carry):
        r = lax.dot_general(q, tiles(wuk_v, u), _NT, preferred_element_type=_F32)
        rows_v[pl.ds(pl.multiple_of(u * TU, TU), TU), :] = jnp.concatenate(
            [jnp.sum(jnp.where(diag, r[:, t * J * H:(t + 1) * J * H], 0.0),
                     axis=0, keepdims=True) for t in range(TU)], axis=0)
        return carry

    lag = NU // 2
    follow_stream(NU, NU + lag, lambda k, c: lax.fori_loop(2 * k, 2 * k + 2, absorb, c), None)
    qt = rows_v[...].T
    qa = jnp.concatenate([qt[j * H:(j + 1) * H, :] for j in range(J)], axis=1)
    qa = (qa * (D ** -0.5)).astype(_BF16)

    def attend(u, carry):
        m, l, acc = carry
        s = lax.dot_general(qa, ckv_v[u], _NT, preferred_element_type=_F32)
        m_new = jnp.maximum(m, jnp.max(s, axis=-1, keepdims=True))
        alpha = jnp.exp(m - m_new)
        p = jnp.exp(s - m_new)
        l = alpha * l + jnp.sum(p, axis=-1, keepdims=True)
        acc = alpha * acc + jnp.dot(p.astype(_BF16), ckv_v[u], preferred_element_type=_F32)
        return m_new, l, acc

    _, l, acc = follow_stream(
        NU + lag, 2 * NU + lag, attend,
        (jnp.full((H, 1), -jnp.inf, _F32), jnp.zeros((H, 1), _F32), jnp.zeros((H, Dc), _F32)))
    lat = acc / l

    rows_v[...] = jnp.concatenate([lat[:, j * T:(j + 1) * T] for j in range(J)], axis=0).T
    contract = functools.partial(head_contract, wuv_v)
    ctx_v[...] = follow_stream(
        2 * NU + lag, 3 * NU,
        lambda k, c: lax.fori_loop(jnp.where(k == 0, 0, lag + k), lag + k + 1, contract, c),
        jnp.zeros((H, D), _F32))

    def out_proj(u, attn):
        for j in range(J):
            a = jnp.broadcast_to(ctx_v[pl.ds(j * NU + u, 1), :], (_ROWS, D)).astype(_BF16)
            attn += jnp.dot(a, wo_v[u, j * D:(j + 1) * D, :], preferred_element_type=_F32)
        return attn

    attn = lax.fori_loop(0, NU, out_proj, jnp.zeros((_ROWS, M), _F32), unroll=2)
    start_ffn(_AHEAD * _UNIT, len(ffn_queue))
    h = x + attn[0:1]
    hn = _layernorm(h)

    cp_wr.wait()
    r = jnp.sum(hn * wr_v[...].astype(_F32).reshape(1, M), axis=-1, keepdims=True)
    gate = jax.nn.sigmoid(r)

    for k, (lo, hi) in enumerate(gu_units):
        wait_ffn(wg_v, lo, hi, 2 * k)
        wait_ffn(wu_v, lo, hi, 2 * k + 1)
        for c in range(lo * _PIECE, hi * _PIECE, _LANES):
            e = min(c + _LANES, hi * _PIECE)
            g = jnp.sum(wg_v[c:e, :].astype(_F32) * hn, axis=-1, keepdims=True)
            up = jnp.sum(wu_v[c:e, :].astype(_F32) * hn, axis=-1, keepdims=True)
            col_v[c:e, :] = jnp.broadcast_to(jax.nn.silu(g) * up * gate, (e - c, _LANES))

    first = lax.broadcasted_iota(jnp.int32, (8, M), 0) == 0
    out = jnp.where(first, h + (hn + hn * 0.0), 0.0)
    out = [out[:, c:c + _LANES] for c in range(0, M, _LANES)]
    for k, (lo, hi) in enumerate(wd_units):
        wait_ffn(wd_v, lo, hi, 2 * len(gu_units) + k)
        for c in range(lo * _PIECE, hi * _PIECE, 16):
            f = gu_order.index(wd_order[c // _PIECE]) * _PIECE + c % _PIECE
            w = wd_v[c:c + 16, :].astype(_F32)
            a = col_v[f:f + 16, :]
            for j in range(M // _LANES):
                t = w[:, j * _LANES:(j + 1) * _LANES] * a
                out[j] = out[j] + (t[0:8] + t[8:16])
    o_ref[0] = jnp.sum(jnp.concatenate(out, axis=1), axis=0, keepdims=True).astype(o_ref.dtype)


@jax.jit
def pallas_sequential_preLN__compressed_kv_cla__moe_arch_mod__decode_kernel(
    A_x: jax.Array,
    A_c_kv: jax.Array,
    A_w_q: jax.Array,
    A_w_uk: jax.Array,
    A_w_uv: jax.Array,
    A_w_o: jax.Array,
    B_x: jax.Array,
    B_w_r: jax.Array,
    B_w_gate: jax.Array,
    B_w_up: jax.Array,
    B_w_down: jax.Array,
):
    del B_x
    B, Sq, M = A_x.shape
    _, Sk, Dc = A_c_kv.shape
    _, H, D = A_w_q.shape
    F = B_w_down.shape[0]
    J = _REGIONS // 2
    NU = Sk // (_UNIT * _PIECE)
    assert (B, Sq) == (1, 1) and M == Dc == J * _LANES and D == J * H == _LANES
    assert Sk == NU * _UNIT * _PIECE and H == J * NU and D == _PER_REGION * _PIECE
    assert F == sum(_GU_UNITS) * _PIECE == sum(_WD_UNITS) * _PIECE
    assert NU % _RING == 0 and _AHEAD < _RING and _AHEAD * _UNIT * _PIECE <= 3 * F
    slabs = (NU, J, _LANES // NU, H, D)
    hbm = pl.BlockSpec(memory_space=pltpu.MemorySpace.HBM)
    return pl.pallas_call(
        _kernel,
        in_specs=[hbm] * 10,
        out_specs=pl.BlockSpec(memory_space=pltpu.MemorySpace.VMEM),
        out_shape=jax.ShapeDtypeStruct((B, Sq, M), A_x.dtype),
        scratch_shapes=[
            pltpu.VMEM((B, Sq, M), _BF16),
            pltpu.VMEM((M,), _BF16),
            pltpu.VMEM(slabs, _BF16),
            pltpu.VMEM(slabs, _BF16),
            pltpu.VMEM((NU, _UNIT * _PIECE, Dc), _BF16),
            pltpu.VMEM(slabs, _BF16),
            pltpu.VMEM((NU, J * D, M), _BF16),
            pltpu.VMEM((F, M), _BF16),
            pltpu.VMEM((F, M), _BF16),
            pltpu.VMEM((F, M), _BF16),
            pltpu.VMEM((_LANES, _LANES), _F32),
            pltpu.VMEM((H, D), _F32),
            pltpu.VMEM((F, _LANES), _F32),
            pltpu.SemaphoreType.DMA((2 * _RING,)),
            pltpu.SemaphoreType.DMA((2,)),
            pltpu.SemaphoreType.DMA((2 * len(_GU_UNITS) + len(_WD_UNITS),)),
        ],
        compiler_params=pltpu.CompilerParams(
            vmem_limit_bytes=64 * 1024 * 1024,
            disable_semaphore_checks=True,
            disable_bounds_checks=True,
        ),
    )(
        A_x, A_c_kv, A_w_q, A_w_uk, A_w_uv, A_w_o, B_w_r,
        B_w_gate.T, B_w_up.T, B_w_down,
    )
```

```python
import functools

import jax
import jax.numpy as jnp
from jax import lax
import jax.experimental.pallas as pl
import jax.experimental.pallas.tpu as pltpu

_F32 = jnp.float32
_BF16 = jnp.bfloat16
_LANES = 128
_NT = (((1,), (1,)), ((), ()))

_PIECE = 32
_REGIONS = 8
_PER_REGION = 4
_UNIT = _REGIONS * _PER_REGION
_AHEAD = 3
_RING = 4
_ROWS = 16

_GU_STRIDE, _GU_UNITS = 16, (16, 16, 11)
_WD_STRIDE, _WD_UNITS = 8, (20, 10, 6, 4, 3)


def _layernorm(x):
    m = jnp.mean(x, axis=-1, keepdims=True)
    d = x - m
    v = jnp.mean(d * d, axis=-1, keepdims=True)
    return d / jnp.sqrt(v + 1e-5)


def _bounds(sizes):
    out, lo = [], 0
    for s in sizes:
        out.append((lo, lo + s))
        lo += s
    return out


def _kernel(
    x_hbm, ckv_hbm, wq_hbm, wuk_hbm, wuv_hbm, wo_hbm, wr_hbm, wg_hbm, wu_hbm, wd_hbm,
    o_ref,
    x_v, wr_v, wq_v, wuk_v, ckv_v, wuv_v, wo_v, wg_v, wu_v, wd_v,
    rows_v, ctx_v, col_v, ring_sems, io_sems, ffn_sems,
):
    NU, J, TU, H, D = wq_v.shape
    Dc = ckv_v.shape[2]
    F, M = wd_v.shape
    T = NU * TU

    def slab_piece(w_hbm, w_v, u, j, i):
        n = TU // _PER_REGION
        return w_hbm.at[pl.ds(j * T + u * TU + i * n, n)], w_v.at[u, j, pl.ds(i * n, n)]

    def wo_piece(u, j, i):
        return (wo_hbm.at[j * NU + u, pl.ds(i * _PIECE, _PIECE)],
                wo_v.at[u, pl.ds(j * D + i * _PIECE, _PIECE)])

    def kv_piece(u, r, i):
        row = ((r * NU + u) * _PER_REGION + i) * _PIECE
        return (ckv_hbm.at[0, pl.ds(pl.multiple_of(row, _PIECE), _PIECE)],
                ckv_v.at[u, pl.ds((r * _PER_REGION + i) * _PIECE, _PIECE)])

    phases = [
        [(functools.partial(slab_piece, wq_hbm, wq_v), wq_v),
         (functools.partial(slab_piece, wuk_hbm, wuk_v), wuk_v)],
        [(kv_piece, ckv_v)],
        [(functools.partial(slab_piece, wuv_hbm, wuv_v), wuv_v), (wo_piece, wo_v)],
    ]
    n_units = len(phases) * NU

    def start_unit(p, u):
        per_array = _REGIONS // len(phases[p])
        for i in range(_PER_REGION):
            for r in range(_REGIONS):
                a = r // per_array
                src, dst = phases[p][a][0](u, r % per_array, i)
                pltpu.make_async_copy(
                    src, dst, ring_sems.at[a * _RING + u % _RING]).start(priority=1 - r % 2)

    def wait_unit(p, u):
        for a, (_, buf) in enumerate(phases[p]):
            pltpu.make_async_copy(
                buf.at[u], buf.at[u], ring_sems.at[a * _RING + u % _RING]).wait()

    def strided(stride):
        return [j for i in range(stride) for j in range(i, F // _PIECE, stride)]

    gu_order, wd_order = strided(_GU_STRIDE), strided(_WD_STRIDE)
    gu_units, wd_units = _bounds(_GU_UNITS), _bounds(_WD_UNITS)
    ffn_queue = []
    for k, (lo, hi) in enumerate(gu_units):
        for i in range(lo, hi):
            ffn_queue += [(wg_hbm, wg_v, gu_order[i], i, 2 * k),
                          (wu_hbm, wu_v, gu_order[i], i, 2 * k + 1)]
    for k, (lo, hi) in enumerate(wd_units):
        ffn_queue += [(wd_hbm, wd_v, wd_order[i], i, 2 * len(gu_units) + k)
                      for i in range(lo, hi)]

    def start_ffn(lo, hi):
        for k in range(lo, hi):
            src, dst, piece, i, s = ffn_queue[k]
            pltpu.make_async_copy(src.at[pl.ds(piece * _PIECE, _PIECE)],
                                  dst.at[pl.ds(i * _PIECE, _PIECE)],
                                  ffn_sems.at[s]).start(priority=1 - k % 2)

    def wait_ffn(buf, lo, hi, s):
        rows = buf.at[pl.ds(lo * _PIECE, (hi - lo) * _PIECE)]
        pltpu.make_async_copy(rows, rows, ffn_sems.at[s]).wait()

    def for_unit(fn, n, lo, hi):
        for p in range(lo // NU, pl.cdiv(min(hi, n_units), NU)):
            if p * NU <= lo and hi <= (p + 1) * NU:
                fn(p, n - p * NU)
            else:
                pl.when((n >= p * NU) & (n < (p + 1) * NU))(
                    lambda p=p: fn(p, n - p * NU))

    def follow_stream(lo, hi, body, init):
        def step(n, carry):
            for_unit(start_unit, n + _AHEAD, lo + _AHEAD, hi + _AHEAD)
            for k in range(max(0, hi + _AHEAD - n_units)):
                pl.when(n + _AHEAD == n_units + k)(
                    functools.partial(start_ffn, k * _UNIT, (k + 1) * _UNIT))
            for_unit(wait_unit, n, lo, hi)
            return body(n - lo, carry)
        return lax.fori_loop(lo, hi, step, init)

    cp_x = pltpu.make_async_copy(x_hbm, x_v, io_sems.at[0])
    cp_wr = pltpu.make_async_copy(wr_hbm, wr_v, io_sems.at[1])
    cp_x.start(priority=1)
    cp_wr.start(priority=0)
    lax.fori_loop(0, _AHEAD, lambda u, c: start_unit(0, u), None)

    diag = (lax.broadcasted_iota(jnp.int32, (H, J * H), 1) % H
            == lax.broadcasted_iota(jnp.int32, (H, J * H), 0))

    def tiles(w_v, u):
        return jnp.concatenate([w_v[u, j, t] for t in range(TU) for j in range(J)], axis=0)

    def head_contract(w_v, u, acc):
        r = rows_v[pl.ds(pl.multiple_of(u * TU, TU), TU), :]
        s = jnp.concatenate(
            [jnp.where(diag, r[t:t + 1, :], 0.0) for t in range(TU)], axis=1)
        return acc + jnp.dot(s.astype(_BF16), tiles(w_v, u), preferred_element_type=_F32)

    cp_x.wait()
    x = x_v[0].astype(_F32)
    xn = _layernorm(x)
    rows_v[...] = jnp.concatenate(
        [jnp.broadcast_to(xn[:, j * T:(j + 1) * T], (H, T)) for j in range(J)], axis=0).T
    q = follow_stream(0, NU, functools.partial(head_contract, wq_v), jnp.zeros((H, D), _F32))
    q = q.astype(_BF16)

    def absorb(u, carry):
        r = lax.dot_general(q, tiles(wuk_v, u), _NT, preferred_element_type=_F32)
        rows_v[pl.ds(pl.multiple_of(u * TU, TU), TU), :] = jnp.concatenate(
            [jnp.sum(jnp.where(diag, r[:, t * J * H:(t + 1) * J * H], 0.0),
                     axis=0, keepdims=True) for t in range(TU)], axis=0)
        return carry

    lag = NU // 2
    follow_stream(NU, NU + lag, lambda k, c: lax.fori_loop(2 * k, 2 * k + 2, absorb, c), None)
    qt = rows_v[...].T
    qa = jnp.concatenate([qt[j * H:(j + 1) * H, :] for j in range(J)], axis=1)
    qa = (qa * (D ** -0.5)).astype(_BF16)

    def attend(u, carry):
        m, l, acc = carry
        s = lax.dot_general(qa, ckv_v[u], _NT, preferred_element_type=_F32)
        m_new = jnp.maximum(m, jnp.max(s, axis=-1, keepdims=True))
        alpha = jnp.exp(m - m_new)
        p = jnp.exp(s - m_new)
        l = alpha * l + jnp.sum(p, axis=-1, keepdims=True)
        acc = alpha * acc + jnp.dot(p.astype(_BF16), ckv_v[u], preferred_element_type=_F32)
        return m_new, l, acc

    _, l, acc = follow_stream(
        NU + lag, 2 * NU + lag, attend,
        (jnp.full((H, 1), -jnp.inf, _F32), jnp.zeros((H, 1), _F32), jnp.zeros((H, Dc), _F32)))
    lat = acc / l

    rows_v[...] = jnp.concatenate([lat[:, j * T:(j + 1) * T] for j in range(J)], axis=0).T
    contract = functools.partial(head_contract, wuv_v)
    ctx_v[...] = follow_stream(
        2 * NU + lag, 3 * NU,
        lambda k, c: lax.fori_loop(jnp.where(k == 0, 0, lag + k), lag + k + 1, contract, c),
        jnp.zeros((H, D), _F32))

    def out_proj(u, attn):
        for j in range(J):
            a = jnp.broadcast_to(ctx_v[pl.ds(j * NU + u, 1), :], (_ROWS, D)).astype(_BF16)
            attn += jnp.dot(a, wo_v[u, j * D:(j + 1) * D, :], preferred_element_type=_F32)
        return attn

    attn = lax.fori_loop(0, NU, out_proj, jnp.zeros((_ROWS, M), _F32), unroll=2)
    start_ffn(_AHEAD * _UNIT, len(ffn_queue))
    h = x + attn[0:1]
    hn = _layernorm(h)

    cp_wr.wait()
    r = jnp.sum(hn * wr_v[...].astype(_F32).reshape(1, M), axis=-1, keepdims=True)
    gate = jax.nn.sigmoid(r)

    for k, (lo, hi) in enumerate(gu_units):
        wait_ffn(wg_v, lo, hi, 2 * k)
        wait_ffn(wu_v, lo, hi, 2 * k + 1)
        for c in range(lo * _PIECE, hi * _PIECE, _LANES):
            e = min(c + _LANES, hi * _PIECE)
            g = jnp.sum(wg_v[c:e, :].astype(_F32) * hn, axis=-1, keepdims=True)
            up = jnp.sum(wu_v[c:e, :].astype(_F32) * hn, axis=-1, keepdims=True)
            col_v[c:e, :] = jnp.broadcast_to(jax.nn.silu(g) * up * gate, (e - c, _LANES))

    first = lax.broadcasted_iota(jnp.int32, (8, M), 0) == 0
    out = jnp.where(first, h + (hn + hn * 0.0), 0.0)
    out = [out[:, c:c + _LANES] for c in range(0, M, _LANES)]
    for k, (lo, hi) in enumerate(wd_units):
        wait_ffn(wd_v, lo, hi, 2 * len(gu_units) + k)
        for c in range(lo * _PIECE, hi * _PIECE, 16):
            f = gu_order.index(wd_order[c // _PIECE]) * _PIECE + c % _PIECE
            w = wd_v[c:c + 16, :].astype(_F32)
            a = col_v[f:f + 16, :]
            for j in range(M // _LANES):
                t = w[:, j * _LANES:(j + 1) * _LANES] * a
                out[j] = out[j] + (t[0:8] + t[8:16])
    o_ref[0] = jnp.sum(jnp.concatenate(out, axis=1), axis=0, keepdims=True).astype(o_ref.dtype)


@jax.jit
def pallas_sequential_preLN__compressed_kv_cla__moe_arch_mod__decode_kernel(
    A_x: jax.Array,
    A_c_kv: jax.Array,
    A_w_q: jax.Array,
    A_w_uk: jax.Array,
    A_w_uv: jax.Array,
    A_w_o: jax.Array,
    B_x: jax.Array,
    B_w_r: jax.Array,
    B_w_gate: jax.Array,
    B_w_up: jax.Array,
    B_w_down: jax.Array,
):
    del B_x
    B, Sq, M = A_x.shape
    _, Sk, Dc = A_c_kv.shape
    _, H, D = A_w_q.shape
    F = B_w_down.shape[0]
    J = _REGIONS // 2
    NU = Sk // (_UNIT * _PIECE)
    assert (B, Sq) == (1, 1) and M == Dc == J * _LANES and D == J * H == _LANES
    assert Sk == NU * _UNIT * _PIECE and H == J * NU and D == _PER_REGION * _PIECE
    assert F == sum(_GU_UNITS) * _PIECE == sum(_WD_UNITS) * _PIECE
    assert NU % _RING == 0 and _AHEAD < _RING and _AHEAD * _UNIT * _PIECE <= 3 * F
    slabs = (NU, J, _LANES // NU, H, D)
    hbm = pl.BlockSpec(memory_space=pltpu.MemorySpace.HBM)
    return pl.pallas_call(
        _kernel,
        in_specs=[hbm] * 10,
        out_specs=pl.BlockSpec(memory_space=pltpu.MemorySpace.VMEM),
        out_shape=jax.ShapeDtypeStruct((B, Sq, M), A_x.dtype),
        scratch_shapes=[
            pltpu.VMEM((B, Sq, M), _BF16),
            pltpu.VMEM((M,), _BF16),
            pltpu.VMEM(slabs, _BF16),
            pltpu.VMEM(slabs, _BF16),
            pltpu.VMEM((NU, _UNIT * _PIECE, Dc), _BF16),
            pltpu.VMEM(slabs, _BF16),
            pltpu.VMEM((NU, J * D, M), _BF16),
            pltpu.VMEM((F, M), _BF16),
            pltpu.VMEM((F, M), _BF16),
            pltpu.VMEM((F, M), _BF16),
            pltpu.VMEM((_LANES, _LANES), _F32),
            pltpu.VMEM((H, D), _F32),
            pltpu.VMEM((F, _LANES), _F32),
            pltpu.SemaphoreType.DMA((2 * _RING,)),
            pltpu.SemaphoreType.DMA((2,)),
            pltpu.SemaphoreType.DMA((2 * len(_GU_UNITS) + len(_WD_UNITS),)),
        ],
        compiler_params=pltpu.CompilerParams(
            vmem_limit_bytes=64 * 1024 * 1024,
            disable_semaphore_checks=True,
            disable_bounds_checks=True,
        ),
    )(
        A_x, A_c_kv, A_w_q, A_w_uk, A_w_uv, A_w_o, B_w_r,
        B_w_gate.T, B_w_up.T, B_w_down,
    )
```
